```python
import os as _os
_os.environ.setdefault("JAX_PLATFORMS", "cpu")
import jax
import jax.numpy as jnp

def _softmax(x, axis=-1):
    return jax.nn.softmax(x, axis=axis)
def _gelu(x):
    return jax.nn.gelu(x, approximate=True)
def _silu(x):
    return jax.nn.silu(x)
def _sigmoid(x):
    return jax.nn.sigmoid(x)
def _layernorm(x, axis=-1, eps=1e-5):
    m = jnp.mean(x, axis=axis, keepdims=True)
    v = jnp.var(x, axis=axis, keepdims=True)
    return (x - m) / jnp.sqrt(v + eps)
def _scatter_add(tgt, idx, src, axis=0):
    return tgt.at[idx].add(src)
def _segment_sum(src, seg, n):
    return jax.ops.segment_sum(src, seg, n)
class _Rng:
    def __init__(self, key):
        self._k = key
    def _next(self):
        self._k, sub = jax.random.split(self._k)
        return sub
    def normal(self, shape):
        return jax.random.normal(self._next(), shape, dtype=jnp.bfloat16)
    def randint(self, lo, hi, shape):
        return jax.random.randint(self._next(), shape, lo, hi, dtype=jnp.int32)
    def uniform(self, shape, lo=0.0, hi=1.0):
        return jax.random.uniform(self._next(), shape, jnp.bfloat16, lo, hi)
    def permutation(self, n):
        return jax.random.permutation(self._next(), n)


kernel_name = 'sequential_preLN__softmax_full_mha__glu_gated_swiglu__prompt'

def setup_inputs():
    _rng = _Rng(jax.random.key(int.from_bytes(__import__("os").urandom(4), "little")))
    _w = (lambda a: (lambda t: t.astype(jnp.bfloat16) if jnp.issubdtype(t.dtype, jnp.floating) else t)(jnp.asarray(a)))
    def _A_setup():
        B, S, D = 1, 2048, 512
        return {
            "x": _w((lambda *s: _rng.normal(s) * 0.05)(B, S, D)),
            "wqkv": _w((lambda *s: _rng.normal(s) * 0.05)(D, 3 * D)),
            "wo": _w((lambda *s: _rng.normal(s) * 0.05)(D, D)),
        }
    _A_in = _A_setup()

    def _B_setup():
        B, S, D, F = 1, 2048, 512, 1376
        return {
            "x": _w((lambda *s: _rng.normal(s) * 0.05)(B, S, D)),
            "w1": _w((lambda *s: _rng.normal(s) * 0.05)(D, F) * (2.0 / D) ** 0.5),
            "w3": _w((lambda *s: _rng.normal(s) * 0.05)(D, F) * (2.0 / D) ** 0.5),
            "w2": _w((lambda *s: _rng.normal(s) * 0.05)(F, D) * (2.0 / F) ** 0.5),
        }
    _B_in = _B_setup()

    return {
        "A_x": _A_in["x"],
        "A_wqkv": _A_in["wqkv"],
        "A_wo": _A_in["wo"],
        "B_x": _B_in["x"],
        "B_w1": _B_in["w1"],
        "B_w3": _B_in["w3"],
        "B_w2": _B_in["w2"],
    }

def reference(A_x, A_wqkv, A_wo, B_x, B_w1, B_w3, B_w2):
    def _A_ref(x, wqkv, wo):
        B, S, D = x.shape
        H = 32; Dh = D // H
        qkv = (lambda x, *d: x.transpose(*d))((x @ wqkv).reshape(B, S, 3, H, Dh), 2, 0, 3, 1, 4)
        q, k, v = qkv[0], qkv[1], qkv[2]
        scale = Dh ** -0.5
        scores = jnp.einsum("bhqd,bhkd->bhqk", q, k) * scale
        p = _softmax(scores, axis=-1)
        o = jnp.einsum("bhqk,bhkd->bhqd", p, v)
        return (lambda x, *d: x.transpose(*d))(o, 0, 2, 1, 3).reshape(B, S, D) @ wo

    def _B_ref(x, w1, w3, w2):
        gate = jnp.einsum("bsd,df->bsf", x, w1)
        up = jnp.einsum("bsd,df->bsf", x, w3)
        h = _silu(gate) * up
        out = jnp.einsum("bsf,fd->bsd", h, w2)
        return out

    x = A_x
    h = x + _A_ref(_layernorm(x, axis=-1), A_wqkv, A_wo)
    h2 = h + _B_ref(_layernorm(h, axis=-1), B_w1, B_w3, B_w2)
    return h2
```

```python
import functools

import jax
import jax.numpy as jnp
from jax import lax
import jax.experimental.pallas as pl
import jax.experimental.pallas.tpu as pltpu

S = 2048
D = 512
H = 32
DH = 16
F = 1376
EPS = 1e-5
LOG2E = 1.4426950408889634
QSCALE = (DH ** -0.5) * LOG2E

TQ = 512
NQ = S // TQ
KC = 128
NC = S // KC
LAG = 2
TM = 512
NM = S // TM

SAFE_BOUND = 80.0
V_HI = 2.0 ** 30
V_LO = 2.0 ** -40

F32 = jnp.float32
BF16 = jnp.bfloat16


def _ln(x):
    m = jnp.mean(x, axis=-1, keepdims=True)
    xc = x - m
    v = jnp.mean(xc * xc, axis=-1, keepdims=True)
    return xc * lax.rsqrt(v + EPS)


def _dot(a, b):
    return jnp.dot(a, b, preferred_element_type=F32)


def _kernel(x_hbm, wqkv_hbm, wo_hbm, w1_hbm, w3_hbm, w2_hbm, out_hbm,
            x_v, wqkv_v, wo_v, w1_v, w3_v, w2_v,
            k_s, qt_s, vt_s, ot_s, out_v, flag_s,
            in_sems, x_sems, out_sems):
    cp_wqkv = pltpu.make_async_copy(wqkv_hbm, wqkv_v, in_sems.at[0])
    cp_wqkv.start()
    cp_x = []
    for b in range(NM):
        c = pltpu.make_async_copy(x_hbm.at[pl.ds(b * TM, TM), :],
                                  x_v.at[pl.ds(b * TM, TM), :], x_sems.at[b])
        c.start()
        cp_x.append(c)
    cp_rest = []
    for i, (src, dst) in enumerate(((wo_hbm, wo_v), (w1_hbm, w1_v),
                                    (w3_hbm, w3_v), (w2_hbm, w2_v))):
        c = pltpu.make_async_copy(src, dst, in_sems.at[i + 1])
        c.start()
        cp_rest.append(c)

    e_rows = lax.broadcasted_iota(jnp.int32, (D, 128), 0) // DH
    e_cols = lax.broadcasted_iota(jnp.int32, (D, 128), 1)
    e_mat = jnp.where(e_rows == e_cols, 1.0, 0.0).astype(BF16)

    cp_wqkv.wait()
    qn_max = jnp.zeros((8, 128), F32)
    kn_max = jnp.zeros((8, 128), F32)
    v_max = jnp.zeros((8, D), F32)
    for b in range(NM):
        cp_x[b].wait()
        xb = x_v[b * TM:(b + 1) * TM, :].astype(F32)
        xn = _ln(xb).astype(BF16)
        q = _dot(xn, wqkv_v[:, 0:D]) * QSCALE
        k = _dot(xn, wqkv_v[:, D:2 * D])
        v = _dot(xn, wqkv_v[:, 2 * D:3 * D])
        qt_s[b] = q.T.astype(BF16)
        kb = k.astype(BF16)
        for g in range(4):
            k_s[g, b * TM:(b + 1) * TM, :] = kb[:, g * 128:(g + 1) * 128]
        vt_s[:, b * TM:(b + 1) * TM] = v.T.astype(BF16)
        qn = _dot((q * q).astype(BF16), e_mat)
        kn = _dot((k * k).astype(BF16), e_mat)
        qn_max = jnp.maximum(qn_max, qn.reshape(TM // 8, 8, 128).max(axis=0))
        kn_max = jnp.maximum(kn_max, kn.reshape(TM // 8, 8, 128).max(axis=0))
        v_max = jnp.maximum(v_max, jnp.abs(v).reshape(TM // 8, 8, D).max(axis=0))
    bound2 = (jnp.max(qn_max, axis=0, keepdims=True)
              * jnp.max(kn_max, axis=0, keepdims=True))
    bound2 = jnp.max(bound2) * 1.05
    vm = jnp.max(v_max)
    safe = jnp.logical_and(bound2 <= SAFE_BOUND * SAFE_BOUND,
                           jnp.logical_and(vm <= V_HI, vm >= V_LO))
    flag_s[0] = safe.astype(jnp.int32)

    zeros16 = jnp.zeros((DH, TQ), BF16)

    def head_weights(qb, g, hh):
        qh = qt_s[qb, pl.ds(pl.multiple_of(g * 128 + hh * DH, DH), DH), :]
        return jnp.concatenate([zeros16] * hh + [qh] + [zeros16] * (7 - hh), axis=0)

    @pl.when(flag_s[0] == 1)
    def _fast():
        def body(it, carry):
            qb = it // 4
            g = it % 4
            items = [(hh, c) for hh in range(8) for c in range(NC)]
            w = {}
            acc = {}
            l = {}
            s = {}

            def qk(i):
                hh, c = items[i]
                if hh not in w:
                    w[hh] = head_weights(qb, g, hh)
                    acc[hh] = jnp.zeros((DH, TQ), F32)
                    l[hh] = jnp.zeros((8, TQ), F32)
                s[i] = _dot(k_s[g, c * KC:(c + 1) * KC, :], w[hh])

            def pv(i):
                hh, c = items[i]
                row = pl.multiple_of(g * 128 + hh * DH, DH)
                p = jnp.exp2(s.pop(i))
                l[hh] = l[hh] + p.reshape(KC // 8, 8, TQ).sum(axis=0)
                vt = vt_s[pl.ds(row, DH), c * KC:(c + 1) * KC]
                acc[hh] = acc[hh] + _dot(vt, p.astype(BF16))
                if c == NC - 1:
                    lsum = l[hh].sum(axis=0, keepdims=True)
                    ot_s[qb, pl.ds(row, DH), :] = acc[hh] * (1.0 / lsum)

            n = len(items)
            for j in range(n + LAG):
                if j < n:
                    qk(j)
                if j >= LAG:
                    pv(j - LAG)
            return carry

        lax.fori_loop(0, NQ * 4, body, 0)

    @pl.when(flag_s[0] != 1)
    def _slow():
        rows = lax.broadcasted_iota(jnp.int32, (128, TQ), 0) // DH

        def body(it, carry):
            qb = it // H
            h = it % H
            g = h // 8
            hh = h % 8
            qg = qt_s[qb, pl.ds(pl.multiple_of(g * 128, 128), 128), :]
            w = jnp.where(rows == hh, qg, jnp.zeros_like(qg))
            s = _dot(k_s[g], w)
            m = jnp.max(s, axis=0, keepdims=True)
            p = jnp.exp2(s - m)
            lsum = jnp.sum(p, axis=0, keepdims=True)
            row = pl.multiple_of(h * DH, DH)
            acc = _dot(vt_s[pl.ds(row, DH), :], p.astype(BF16))
            ot_s[qb, pl.ds(row, DH), :] = acc * (1.0 / lsum)
            return carry

        lax.fori_loop(0, NQ * H, body, 0)

    for c in cp_rest:
        c.wait()
    cp_out = []
    for b in range(NM):
        o = ot_s[b].T.astype(BF16)
        h = x_v[b * TM:(b + 1) * TM, :].astype(F32) + _dot(o, wo_v[...])
        hn = _ln(h).astype(BF16)
        gate = _dot(hn, w1_v[...])
        up = _dot(hn, w3_v[...])
        a = (gate * jax.nn.sigmoid(gate) * up).astype(BF16)
        y = h + _dot(a, w2_v[...])
        out_v[b * TM:(b + 1) * TM, :] = y.astype(BF16)
        c = pltpu.make_async_copy(out_v.at[pl.ds(b * TM, TM), :],
                                  out_hbm.at[pl.ds(b * TM, TM), :], out_sems.at[b])
        c.start()
        cp_out.append(c)
    for c in cp_out:
        c.wait()


@jax.jit
def pallas_sequential_preLN__softmax_full_mha__glu_gated_swiglu__prompt_kernel(
    A_x: jax.Array,
    A_wqkv: jax.Array,
    A_wo: jax.Array,
    B_x: jax.Array,
    B_w1: jax.Array,
    B_w3: jax.Array,
    B_w2: jax.Array,
):
    del B_x
    x = A_x.reshape(S, D)
    any_spec = pl.BlockSpec(memory_space=pl.ANY)
    out = pl.pallas_call(
        _kernel,
        out_shape=jax.ShapeDtypeStruct((S, D), BF16),
        in_specs=[any_spec] * 6,
        out_specs=any_spec,
        scratch_shapes=[
            pltpu.VMEM((S, D), BF16),
            pltpu.VMEM((D, 3 * D), BF16),
            pltpu.VMEM((D, D), BF16),
            pltpu.VMEM((D, F), BF16),
            pltpu.VMEM((D, F), BF16),
            pltpu.VMEM((F, D), BF16),
            pltpu.VMEM((4, S, 128), BF16),
            pltpu.VMEM((NQ, D, TQ), BF16),
            pltpu.VMEM((D, S), BF16),
            pltpu.VMEM((NQ, D, TQ), F32),
            pltpu.VMEM((S, D), BF16),
            pltpu.SMEM((1,), jnp.int32),
            pltpu.SemaphoreType.DMA((5,)),
            pltpu.SemaphoreType.DMA((NM,)),
            pltpu.SemaphoreType.DMA((NM,)),
        ],
        compiler_params=pltpu.CompilerParams(vmem_limit_bytes=100 * 1024 * 1024),
        name="preln_mha_swiglu",
    )(x, A_wqkv, A_wo, B_w1, B_w3, B_w2)
    return out.reshape(1, S, D)
```

```python
import functools

import jax
import jax.numpy as jnp
from jax import lax
import jax.experimental.pallas as pl
import jax.experimental.pallas.tpu as pltpu

S = 2048
D = 512
H = 32
DH = 16
F = 1376
EPS = 1e-5
LOG2E = 1.4426950408889634
QSCALE = (DH ** -0.5) * LOG2E

TQ = 512
NQ = S // TQ
KC = 128
NC = S // KC
LAG = 2
TM = 512
NM = S // TM
NSPLIT = 4
NG = D // 128

OFF = 16
KM = KC - OFF
K_TINY = 2.0 ** -50
SAFE_BOUND = 80.0
QN_HI = 2.0 ** 40
KN_HI = 2.0 ** 60
V_HI = 2.0 ** 30
V_LO = 2.0 ** -40

F32 = jnp.float32
BF16 = jnp.bfloat16
NT = (((1,), (1,)), ((), ()))


def _ln(x):
    m = jnp.mean(x, axis=-1, keepdims=True)
    xc = x - m
    v = jnp.mean(xc * xc, axis=-1, keepdims=True)
    return xc * lax.rsqrt(v + EPS)


def _dot(a, b):
    return jnp.dot(a, b, preferred_element_type=F32)


def _dot_nt(a, b):
    return lax.dot_general(a, b, NT, preferred_element_type=F32)


def _kernel(x_hbm, wqkv_hbm, wo_hbm, w1t_hbm, w3t_hbm, w2_hbm, out_hbm,
            x_v, wqkv_v, wo_v, w1t_v, w3t_v, w2_v,
            xn_s, k_s, rt_s, qt_s, ksq_s, vt_s, ot_s, cs_s, cacc_s, out_v, stat_s, flag_s,
            w_sems, x_sems, out_sems):
    scope = jax.named_scope

    def x_copy(b):
        return pltpu.make_async_copy(x_hbm.at[pl.ds(b * TM, TM), :],
                                     x_v.at[pl.ds(b * TM, TM), :], x_sems.at[b])

    def w_copy(j):
        return pltpu.make_async_copy(wqkv_hbm.at[:, pl.ds(j * D, D)],
                                     wqkv_v.at[:, pl.ds(j * D, D)], w_sems.at[j])

    cp_x = [x_copy(b) for b in range(NM)]
    cp_w = [w_copy(j) for j in range(3)]
    cp_rest = [pltpu.make_async_copy(src, dst, w_sems.at[3 + i])
               for i, (src, dst) in enumerate(((wo_hbm, wo_v), (w1t_hbm, w1t_v),
                                               (w3t_hbm, w3t_v), (w2_hbm, w2_v)))]

    et_rows = lax.broadcasted_iota(jnp.int32, (H, D), 0)
    et_cols = lax.broadcasted_iota(jnp.int32, (H, D), 1) // DH
    et = jnp.where(et_rows == et_cols, 1.0, 0.0).astype(BF16)

    def rows(b):
        return pl.ds(pl.multiple_of(b * TM, TM), TM)

    def ln1(b):
        xn_s[rows(b), :] = _ln(x_v[rows(b), :].astype(F32)).astype(BF16)

    def run_max(slot, nrow, val):
        m = stat_s[slot, 0:nrow, :]
        for j in range(TM // 128):
            m = jnp.maximum(m, val[:, j * 128:(j + 1) * 128])
        stat_s[slot, 0:nrow, :] = m

    def proj_k(b):
        k = _dot(xn_s[rows(b), :], wqkv_v[:, D:2 * D])
        kb = k.astype(BF16)
        half = pl.ds(pl.multiple_of(b * (TM // 2), TM // 2), TM // 2)
        lane = lax.broadcasted_iota(jnp.int32, (OFF, 128), 1)
        for g in range(NG):
            kg = kb[:, g * 128:(g + 1) * 128]
            k_s[g, half, :] = pltpu.bitcast(kg, jnp.uint32)
            for j in range(TM // KC):
                kk = kg[j * KC + KM:(j + 1) * KC, :].astype(F32)
                kk = jnp.where(jnp.abs(kk) < K_TINY, K_TINY, kk)
                ratio = kk / pltpu.roll(kk, 1, 1)
                r0 = pl.multiple_of((b * (TM // KC) + j) * OFF, OFF)
                rt_s[g, pl.ds(r0, OFF), :] = jnp.where(lane % DH == 0, kk, ratio)
        ksq_s[...] = (k * k).astype(BF16)

    def proj_q(b):
        qt = (_dot(xn_s[rows(b), :], wqkv_v[:, 0:D]) * QSCALE).T
        qt_s[b] = qt.astype(BF16)
        return (qt * qt).astype(BF16)

    def proj_v(b):
        vt = _dot(xn_s[rows(b), :], wqkv_v[:, 2 * D:3 * D]).T
        vt_s[b] = vt.astype(BF16)
        run_max(2, 8, jnp.abs(vt).reshape(D // 8, 8, TM).max(axis=0))

    def norm_k():
        run_max(0, H, _dot_nt(et, ksq_s[...]))

    def norm_q(qsq):
        run_max(1, H, _dot(et, qsq))

    cp_x[0].start()
    cp_w[0].start()
    stat_s[...] = jnp.zeros(stat_s.shape, F32)
    with scope('wait_x0'):
        cp_x[0].wait()
    cp_w[2].start()
    ln1(0)
    with scope('wait_wq'):
        cp_w[0].wait()
    cp_w[1].start()
    cp_x[1].start()
    qsq0 = proj_q(0)
    with scope('wait_wv'):
        cp_w[2].wait()
    cp_x[2].start()
    cp_x[3].start()
    proj_v(0)
    norm_q(qsq0)
    with scope('wait_x1'):
        cp_w[1].wait()
        cp_x[1].wait()
    proj_k(0)
    ln1(1)
    with scope('wait_x23'):
        cp_x[2].wait()
        cp_x[3].wait()
    for c in cp_rest:
        c.start()

    def a_body(b, carry):
        qsq = proj_q(b)
        norm_k()
        proj_v(b)
        norm_q(qsq)
        proj_k(b)
        ln1(jnp.minimum(b + 1, NM - 1))
        return carry

    lax.fori_loop(1, NM, scope('a_iter')(a_body), 0)
    norm_k()
    bound2 = (jnp.max(stat_s[0], axis=1, keepdims=True)
              * jnp.max(stat_s[1], axis=1, keepdims=True))
    bound2 = jnp.max(bound2) * 1.05
    vm = jnp.max(stat_s[2, 0:8, :])
    safe = jnp.logical_and(bound2 <= SAFE_BOUND * SAFE_BOUND,
                           jnp.logical_and(vm <= V_HI, vm >= V_LO))
    safe = jnp.logical_and(safe, jnp.logical_and(jnp.max(stat_s[1]) <= QN_HI,
                                                 jnp.max(stat_s[0]) <= KN_HI))
    with scope('flag'):
        flag_s[0] = safe.astype(jnp.int32)

    zeros16 = jnp.zeros((DH, TQ), BF16)

    def head_weights(qb, g, hh):
        qh = qt_s[qb, pl.ds(pl.multiple_of(g * 128 + hh * DH, DH), DH), :]
        return jnp.concatenate([zeros16] * hh + [qh] + [zeros16] * (7 - hh), axis=0)

    def vt_chunk(row, c):
        k0 = (c * KC) % TM
        return vt_s[(c * KC) // TM, pl.ds(row, DH), k0:k0 + KC]

    def pv_step(s, row, c, acc, l):
        p = jnp.exp2(s)
        l = l + p.reshape(KC // 8, 8, TQ).sum(axis=0)
        acc = acc + _dot(vt_chunk(row, c), p.astype(BF16))
        return acc, l

    def finish(slot, hh, acc, l):
        lsum = l.sum(axis=0, keepdims=True)
        ot_s[slot, hh * DH:(hh + 1) * DH, :] = acc * (1.0 / lsum)

    @pl.when(flag_s[0] == 1)
    def _fast():
        def tail(it_prev, slot_prev):
            row = pl.multiple_of((it_prev % NG) * 128 + 7 * DH, DH)
            acc = cacc_s[0:DH, :]
            l = cacc_s[DH:DH + 8, :]
            for j in range(LAG):
                acc, l = pv_step(cs_s[j], row, NC - LAG + j, acc, l)
                yield None
            finish(slot_prev, 7, acc, l)
            yield None

        def body(it, carry):
            qb = it // NG
            g = it % NG
            items = [(hh, c) for hh in range(8) for c in range(NC)]
            n = len(items)
            w = {}
            qrow = {}
            acc = {}
            l = {}
            s = {}

            def qk(i):
                hh, c = items[i]
                if hh not in w:
                    w[hh] = head_weights(qb, g, hh)
                    qf = w[hh][hh * DH:(hh + 1) * DH, :].astype(F32)
                    qrow[hh] = [jnp.broadcast_to(qf[d:d + 1, :], (8, TQ)) for d in range(DH)]
                    acc[hh] = jnp.zeros((DH, TQ), F32)
                    l[hh] = jnp.zeros((8, TQ), F32)
                p0 = c * (KC // 2)
                km = pltpu.bitcast(k_s[g, p0:p0 + KM // 2, :], BF16)
                sm = _dot(km, w[hh])
                r = rt_s[g, c * OFF:(c + 1) * OFF, :]
                a = [qrow[hh][DH - 1]] * (OFF // 8)
                for d in range(DH - 1, -1, -1):
                    rb = jnp.broadcast_to(r[:, hh * DH + d:hh * DH + d + 1], (OFF, TQ))
                    a = [a[u] * rb[u * 8:(u + 1) * 8] for u in range(OFF // 8)]
                    if d > 0:
                        a = [x + qrow[hh][d - 1] for x in a]
                sc = jnp.concatenate([sm] + a, axis=0)
                if i >= n - LAG:
                    cs_s[i - (n - LAG)] = sc
                else:
                    s[i] = sc

            def pv(i):
                hh, c = items[i]
                row = pl.multiple_of(g * 128 + hh * DH, DH)
                acc[hh], l[hh] = pv_step(s.pop(i), row, c, acc[hh], l[hh])
                if c == NC - 1:
                    finish(it, hh, acc[hh], l[hh])

            prev = tail(jnp.maximum(it - 1, 0), jnp.where(it == 0, NQ * NG, it - 1))
            for j in range(n):
                qk(j)
                if j >= LAG:
                    pv(j - LAG)
                else:
                    next(prev)
                    if j == LAG - 1:
                        next(prev)
            cacc_s[0:DH, :] = acc[7]
            cacc_s[DH:DH + 8, :] = l[7]
            return carry

        cs_s[...] = jnp.zeros(cs_s.shape, F32)
        cacc_s[...] = jnp.zeros(cacc_s.shape, F32)
        lax.fori_loop(0, NQ * NG, scope('attn_iter')(body), 0)
        for _ in tail(NQ * NG - 1, NQ * NG - 1):
            pass

    @pl.when(flag_s[0] != 1)
    def _slow():
        def body(it, carry):
            qb = it // H
            h = it % H
            g = h // 8
            hh = h % 8
            qg = qt_s[qb, pl.ds(pl.multiple_of(g * 128, 128), 128), :]
            head_rows = lax.broadcasted_iota(jnp.int32, (128, TQ), 0) // DH
            s = _dot(pltpu.bitcast(k_s[g], BF16),
                     jnp.where(head_rows == hh, qg, jnp.zeros_like(qg)))
            m = jnp.max(s, axis=0, keepdims=True)
            p = jnp.exp2(s - m)
            lsum = jnp.sum(p, axis=0, keepdims=True)
            pb = p.astype(BF16)
            row = pl.multiple_of(h * DH, DH)
            acc = jnp.zeros((DH, TQ), F32)
            for b in range(NM):
                acc = acc + _dot(vt_s[b, pl.ds(row, DH), :], pb[b * TM:(b + 1) * TM])
            ot_s[qb * NG + g, pl.ds(pl.multiple_of(hh * DH, DH), DH), :] = acc * (1.0 / lsum)
            return carry

        lax.fori_loop(0, NQ * H, body, 0)

    with scope('rest_wait'):
        for c in cp_rest:
            c.wait()

    def out_copy(b):
        return pltpu.make_async_copy(out_v.at[rows(b), :], out_hbm.at[rows(b), :],
                                     out_sems.at[b])

    def c_body(b, carry):
        hs = []
        hns = []
        for j in range(NSPLIT):
            tr = TM // NSPLIT
            o = ot_s[pl.ds(b * NG, NG), :, j * tr:(j + 1) * tr].reshape(D, tr).T.astype(BF16)
            xr = x_v[pl.ds(pl.multiple_of(b * TM + j * tr, tr), tr), :].astype(F32)
            hj = xr + _dot(o, wo_v[...])
            hs.append(hj)
            hns.append(_ln(hj).astype(BF16))
        h = jnp.concatenate(hs, axis=0)
        hn = jnp.concatenate(hns, axis=0)
        gate = _dot_nt(hn, w1t_v[...])
        up = _dot_nt(hn, w3t_v[...])
        a = (gate * jax.nn.sigmoid(gate) * up).astype(BF16)
        y = h + _dot(a, w2_v[...])
        out_v[rows(b), :] = y.astype(BF16)
        out_copy(b).start()
        return carry

    lax.fori_loop(0, NM, scope('c_iter')(c_body), 0)
    with scope('out_wait'):
        for b in range(NM):
            out_copy(b).wait()


@jax.jit
def pallas_sequential_preLN__softmax_full_mha__glu_gated_swiglu__prompt_kernel(
    A_x: jax.Array,
    A_wqkv: jax.Array,
    A_wo: jax.Array,
    B_x: jax.Array,
    B_w1: jax.Array,
    B_w3: jax.Array,
    B_w2: jax.Array,
):
    del B_x
    x = A_x.reshape(S, D)
    hbm_spec = pl.BlockSpec(memory_space=pltpu.HBM)
    out = pl.pallas_call(
        _kernel,
        out_shape=jax.ShapeDtypeStruct((S, D), BF16),
        in_specs=[hbm_spec] * 6,
        out_specs=hbm_spec,
        scratch_shapes=[
            pltpu.VMEM((S, D), BF16),
            pltpu.VMEM((D, 3 * D), BF16),
            pltpu.VMEM((D, D), BF16),
            pltpu.VMEM((F, D), BF16),
            pltpu.VMEM((F, D), BF16),
            pltpu.VMEM((F, D), BF16),
            pltpu.VMEM((S, D), BF16),
            pltpu.VMEM((NG, S // 2, 128), jnp.uint32),
            pltpu.VMEM((NG, NC * OFF, 128), F32),
            pltpu.VMEM((NQ, D, TQ), BF16),
            pltpu.VMEM((TM, D), BF16),
            pltpu.VMEM((NM, D, TM), BF16),
            pltpu.VMEM((NQ * NG + 1, 128, TQ), F32),
            pltpu.VMEM((LAG, KC, TQ), F32),
            pltpu.VMEM((DH + 8, TQ), F32),
            pltpu.VMEM((S, D), BF16),
            pltpu.VMEM((3, H, 128), F32),
            pltpu.SMEM((1,), jnp.int32),
            pltpu.SemaphoreType.DMA((7,)),
            pltpu.SemaphoreType.DMA((NM,)),
            pltpu.SemaphoreType.DMA((NM,)),
        ],
        compiler_params=pltpu.CompilerParams(vmem_limit_bytes=100 * 1024 * 1024),
        name="preln_mha_swiglu",
    )(x, A_wqkv, A_wo, B_w1.T, B_w3.T, B_w2)
    return out.reshape(1, S, D)
```

```python
import jax
import jax.numpy as jnp
from jax import lax
import jax.experimental.pallas as pl
import jax.experimental.pallas.tpu as pltpu

S = 2048
D = 512
H = 32
DH = 16
F = 1376
EPS = 1e-5
LOG2E = 1.4426950408889634
QSCALE = (DH ** -0.5) * LOG2E

TQ = 512
NQ = S // TQ
KC = 128
NC = S // KC
LAG = 2
TM = 512
NM = S // TM
NSPLIT = 4
TO = 128
NG = D // 128
HG = 128 // DH

OFF = 16
KM = KC - OFF

SAFE_BOUND = 80.0
QN_HI = 2.0 ** 40
KN_HI = 2.0 ** 60
V_HI = 2.0 ** 30
V_LO = 2.0 ** -20
K_TINY = 2.0 ** -50

F32 = jnp.float32
BF16 = jnp.bfloat16
NT = (((1,), (1,)), ((), ()))


def _ln(x):
    m = jnp.mean(x, axis=-1, keepdims=True)
    xc = x - m
    v = jnp.mean(xc * xc, axis=-1, keepdims=True)
    return xc * lax.rsqrt(v + EPS)


def _dot(a, b):
    return jnp.dot(a, b, preferred_element_type=F32)


def _dot_nt(a, b):
    return lax.dot_general(a, b, NT, preferred_element_type=F32)


def _kernel(x_hbm, wqkv_hbm, wo_hbm, w1t_hbm, w3t_hbm, w2_hbm, out_hbm,
            x_v, wqkv_v, wo_v, w1t_v, w3t_v, w2_v,
            xn_s, k_s, rt_s, qt_s, vt_s, ot_s, cs_s, cacc_s, out_v, stat_s, flag_s,
            w_sems, x_sems, out_sems):
    def x_copy(b):
        return pltpu.make_async_copy(x_hbm.at[pl.ds(b * TM, TM), :],
                                     x_v.at[pl.ds(b * TM, TM), :], x_sems.at[b])

    def w_copy(j):
        return pltpu.make_async_copy(wqkv_hbm.at[:, pl.ds(j * D, D)],
                                     wqkv_v.at[:, pl.ds(j * D, D)], w_sems.at[j])

    cp_x = [x_copy(b) for b in range(NM)]
    cp_w = [w_copy(j) for j in range(3)]
    cp_rest = [pltpu.make_async_copy(src, dst, w_sems.at[3 + i])
               for i, (src, dst) in enumerate(((wo_hbm, wo_v), (w1t_hbm, w1t_v),
                                               (w3t_hbm, w3t_v), (w2_hbm, w2_v)))]

    et_rows = lax.broadcasted_iota(jnp.int32, (H, D), 0)
    et_cols = lax.broadcasted_iota(jnp.int32, (H, D), 1) // DH
    et = jnp.where(et_rows == et_cols, 1.0, 0.0).astype(BF16)

    def rows(b):
        return pl.ds(pl.multiple_of(b * TM, TM), TM)

    def ln1(b):
        xn_s[rows(b), :] = _ln(x_v[rows(b), :].astype(F32)).astype(BF16)

    def run_max(slot, nrow, val):
        m = stat_s[slot, 0:nrow, :]
        for j in range(TM // 128):
            m = jnp.maximum(m, val[:, j * 128:(j + 1) * 128])
        stat_s[slot, 0:nrow, :] = m

    def proj_k(b):
        k = _dot(xn_s[rows(b), :], wqkv_v[:, D:2 * D])
        kb = k.astype(BF16)
        half = pl.ds(pl.multiple_of(b * (TM // 2), TM // 2), TM // 2)
        lane = lax.broadcasted_iota(jnp.int32, (OFF, 128), 1)
        for g in range(NG):
            kg = kb[:, g * 128:(g + 1) * 128]
            k_s[g, half, :] = pltpu.bitcast(kg, jnp.uint32)
            for j in range(TM // KC):
                kk = kg[j * KC + KM:(j + 1) * KC, :].astype(F32)
                kk = jnp.where(jnp.abs(kk) < K_TINY, K_TINY, kk)
                ratio = kk / pltpu.roll(kk, 1, 1)
                r0 = pl.multiple_of((b * (TM // KC) + j) * OFF, OFF)
                rt_s[g, pl.ds(r0, OFF), :] = jnp.where(lane % DH == 0, kk, ratio)
        return (k * k).astype(BF16)

    def proj_q(b):
        qt = (_dot(xn_s[rows(b), :], wqkv_v[:, 0:D]) * QSCALE).T
        qt_s[b] = qt.astype(BF16)
        return (qt * qt).astype(BF16)

    def proj_v(b):
        vt = _dot(xn_s[rows(b), :], wqkv_v[:, 2 * D:3 * D]).T
        vt_s[b] = vt.astype(BF16)
        run_max(2, 8, jnp.abs(vt).reshape(D // 8, 8, TM).max(axis=0))

    def norm_k(ksq):
        run_max(0, H, _dot_nt(et, ksq))

    def norm_q(qsq):
        run_max(1, H, _dot(et, qsq))

    cp_x[0].start()
    cp_w[1].start()
    stat_s[...] = jnp.zeros(stat_s.shape, F32)
    cp_x[0].wait()
    cp_w[0].start()
    ln1(0)
    cp_w[1].wait()
    cp_w[2].start()
    cp_x[1].start()
    ksq0 = proj_k(0)
    cp_w[0].wait()
    cp_x[2].start()
    cp_x[3].start()
    qsq0 = proj_q(0)
    norm_k(ksq0)
    cp_w[2].wait()
    cp_x[1].wait()
    proj_v(0)
    norm_q(qsq0)
    ln1(1)
    cp_x[2].wait()
    cp_x[3].wait()
    for c in cp_rest:
        c.start()

    for b in range(1, NM):
        ksq = proj_k(b)
        qsq = proj_q(b)
        norm_k(ksq)
        proj_v(b)
        norm_q(qsq)
        if b + 1 < NM:
            ln1(b + 1)

    zeros16 = jnp.zeros((DH, TQ), BF16)

    def head_weights(qb, g, hh):
        qh = qt_s[qb, pl.ds(pl.multiple_of(g * 128 + hh * DH, DH), DH), :]
        return qh, jnp.concatenate([zeros16] * hh + [qh] + [zeros16] * (HG - 1 - hh), axis=0)

    def pv_step(s, row, c, acc, l):
        p = jnp.exp2(s)
        l = l + p.reshape(KC // 8, 8, TQ).sum(axis=0)
        k0 = (c * KC) % TM
        vt = vt_s[(c * KC) // TM, pl.ds(row, DH), k0:k0 + KC]
        return acc + _dot(vt, p.astype(BF16)), l

    def finish(slot, hh, acc, l):
        lsum = l.sum(axis=0, keepdims=True)
        ot_s[slot, hh * DH:(hh + 1) * DH, :] = acc * (1.0 / lsum)

    def tail(it_prev, slot_prev):
        row = pl.multiple_of((it_prev % NG) * 128 + (HG - 1) * DH, DH)
        acc = cacc_s[0:DH, :]
        l = cacc_s[DH:DH + 8, :]
        for j in range(LAG):
            acc, l = pv_step(cs_s[j], row, NC - LAG + j, acc, l)
            yield None
        finish(slot_prev, HG - 1, acc, l)
        yield None

    def b_body(it, carry):
        qb = it // NG
        g = it % NG
        items = [(hh, c) for hh in range(HG) for c in range(NC)]
        n = len(items)
        w = {}
        qrow = {}
        acc = {}
        l = {}
        s = {}

        def qk(i):
            hh, c = items[i]
            if hh not in w:
                qh, w[hh] = head_weights(qb, g, hh)
                qf = qh.astype(F32)
                qrow[hh] = [jnp.broadcast_to(qf[d:d + 1, :], (8, TQ)) for d in range(DH)]
                acc[hh] = jnp.zeros((DH, TQ), F32)
                l[hh] = jnp.zeros((8, TQ), F32)
            p0 = c * (KC // 2)
            km = pltpu.bitcast(k_s[g, p0:p0 + KM // 2, :], BF16)
            sm = _dot(km, w[hh])
            r = rt_s[g, c * OFF:(c + 1) * OFF, :]
            a = [qrow[hh][DH - 1]] * (OFF // 8)
            for d in range(DH - 1, -1, -1):
                rb = jnp.broadcast_to(r[:, hh * DH + d:hh * DH + d + 1], (OFF, TQ))
                a = [a[u] * rb[u * 8:(u + 1) * 8] for u in range(OFF // 8)]
                if d > 0:
                    a = [x + qrow[hh][d - 1] for x in a]
            sc = jnp.concatenate([sm] + a, axis=0)
            if i >= n - LAG:
                cs_s[i - (n - LAG)] = sc
            else:
                s[i] = sc

        def pv(i):
            hh, c = items[i]
            row = pl.multiple_of(g * 128 + hh * DH, DH)
            acc[hh], l[hh] = pv_step(s.pop(i), row, c, acc[hh], l[hh])
            if c == NC - 1:
                finish(it, hh, acc[hh], l[hh])

        prev = tail(jnp.maximum(it - 1, 0), jnp.where(it == 0, NQ * NG, it - 1))
        for j in range(n):
            qk(j)
            if j >= LAG:
                pv(j - LAG)
            else:
                next(prev)
                if j == LAG - 1:
                    next(prev)
        cacc_s[0:DH, :] = acc[HG - 1]
        cacc_s[DH:DH + 8, :] = l[HG - 1]
        return carry

    cs_s[...] = jnp.zeros(cs_s.shape, F32)
    cacc_s[...] = jnp.zeros(cacc_s.shape, F32)
    lax.fori_loop(0, NQ * NG, b_body, 0)
    for _ in tail(NQ * NG - 1, NQ * NG - 1):
        pass

    bound2 = (jnp.max(stat_s[0], axis=1, keepdims=True)
              * jnp.max(stat_s[1], axis=1, keepdims=True))
    bound2 = jnp.max(bound2) * 1.05
    vm = jnp.max(stat_s[2, 0:8, :])
    safe = jnp.logical_and(bound2 <= SAFE_BOUND * SAFE_BOUND,
                           jnp.logical_and(vm <= V_HI, vm >= V_LO))
    safe = jnp.logical_and(safe, jnp.logical_and(jnp.max(stat_s[1]) <= QN_HI,
                                                 jnp.max(stat_s[0]) <= KN_HI))
    flag_s[0] = safe.astype(jnp.int32)

    @pl.when(flag_s[0] != 1)
    def _true_max_attention():
        head_rows = lax.broadcasted_iota(jnp.int32, (128, TQ), 0) // DH

        def body(it, carry):
            qb = it // H
            h = it % H
            g = h // HG
            hh = h % HG
            qg = qt_s[qb, pl.ds(pl.multiple_of(g * 128, 128), 128), :]
            w = jnp.where(head_rows == hh, qg, jnp.zeros_like(qg))
            row = pl.multiple_of(h * DH, DH)

            def scores(c):
                p0 = pl.multiple_of(c * (TM // 2), TM // 2)
                return _dot(pltpu.bitcast(k_s[g, pl.ds(p0, TM // 2), :], BF16), w)

            def max_pass(c, m):
                return jnp.maximum(m, jnp.max(scores(c), axis=0, keepdims=True))

            m = lax.fori_loop(0, NM, max_pass, jnp.full((1, TQ), -jnp.inf, F32))

            def sum_pass(c, al):
                acc, lsum = al
                p = jnp.exp2(scores(c) - m)
                return (acc + _dot(vt_s[c, pl.ds(row, DH), :], p.astype(BF16)),
                        lsum + jnp.sum(p, axis=0, keepdims=True))

            acc, lsum = lax.fori_loop(
                0, NM, sum_pass, (jnp.zeros((DH, TQ), F32), jnp.zeros((1, TQ), F32)))
            ot_s[qb * NG + g, pl.ds(pl.multiple_of(hh * DH, DH), DH), :] = acc * (1.0 / lsum)
            return carry

        lax.fori_loop(0, NQ * H, body, 0)

    for c in cp_rest:
        c.wait()

    def out_copy(b, j):
        r = pl.ds(pl.multiple_of(b * TM + j * TO, TO), TO)
        return pltpu.make_async_copy(out_v.at[r, :], out_hbm.at[r, :],
                                     out_sems.at[b * (TM // TO) + j])

    def c_body(b, carry):
        hs = []
        hns = []
        tr = TM // NSPLIT
        for j in range(NSPLIT):
            o = ot_s[pl.ds(b * NG, NG), :, j * tr:(j + 1) * tr].reshape(D, tr).T.astype(BF16)
            xr = x_v[pl.ds(pl.multiple_of(b * TM + j * tr, tr), tr), :].astype(F32)
            hj = xr + _dot(o, wo_v[...])
            hs.append(hj)
            hns.append(_ln(hj).astype(BF16))
        h = jnp.concatenate(hs, axis=0)
        hn = jnp.concatenate(hns, axis=0)
        gate = _dot_nt(hn, w1t_v[...])
        up = _dot_nt(hn, w3t_v[...])
        a = (gate * jax.nn.sigmoid(gate) * up).astype(BF16)
        for j in range(TM // TO):
            y = h[j * TO:(j + 1) * TO] + _dot(a[j * TO:(j + 1) * TO], w2_v[...])
            out_v[pl.ds(pl.multiple_of(b * TM + j * TO, TO), TO), :] = y.astype(BF16)
            out_copy(b, j).start()
        return carry

    lax.fori_loop(0, NM, c_body, 0)
    for b in range(NM):
        for j in range(TM // TO):
            out_copy(b, j).wait()


@jax.jit
def pallas_sequential_preLN__softmax_full_mha__glu_gated_swiglu__prompt_kernel(
    A_x: jax.Array,
    A_wqkv: jax.Array,
    A_wo: jax.Array,
    B_x: jax.Array,
    B_w1: jax.Array,
    B_w3: jax.Array,
    B_w2: jax.Array,
):
    del B_x
    x = A_x.reshape(S, D)
    hbm_spec = pl.BlockSpec(memory_space=pltpu.HBM)
    out = pl.pallas_call(
        _kernel,
        out_shape=jax.ShapeDtypeStruct((S, D), BF16),
        in_specs=[hbm_spec] * 6,
        out_specs=hbm_spec,
        scratch_shapes=[
            pltpu.VMEM((S, D), BF16),
            pltpu.VMEM((D, 3 * D), BF16),
            pltpu.VMEM((D, D), BF16),
            pltpu.VMEM((F, D), BF16),
            pltpu.VMEM((F, D), BF16),
            pltpu.VMEM((F, D), BF16),
            pltpu.VMEM((S, D), BF16),
            pltpu.VMEM((NG, S // 2, 128), jnp.uint32),
            pltpu.VMEM((NG, NC * OFF, 128), F32),
            pltpu.VMEM((NQ, D, TQ), BF16),
            pltpu.VMEM((NM, D, TM), BF16),
            pltpu.VMEM((NQ * NG + 1, 128, TQ), F32),
            pltpu.VMEM((LAG, KC, TQ), F32),
            pltpu.VMEM((DH + 8, TQ), F32),
            pltpu.VMEM((S, D), BF16),
            pltpu.VMEM((3, H, 128), F32),
            pltpu.SMEM((1,), jnp.int32),
            pltpu.SemaphoreType.DMA((7,)),
            pltpu.SemaphoreType.DMA((NM,)),
            pltpu.SemaphoreType.DMA((S // TO,)),
        ],
        compiler_params=pltpu.CompilerParams(vmem_limit_bytes=100 * 1024 * 1024),
        name="preln_mha_swiglu",
    )(x, A_wqkv, A_wo, B_w1.T, B_w3.T, B_w2)
    return out.reshape(1, S, D)
```

```python
import jax
import jax.numpy as jnp
from jax import lax
import jax.experimental.pallas as pl
import jax.experimental.pallas.tpu as pltpu

S = 2048
D = 512
H = 32
DH = 16
F = 1376
EPS = 1e-5
LOG2E = 1.4426950408889634
QSCALE = (DH ** -0.5) * LOG2E

TQ = 512
NQ = S // TQ
KC = 128
NC = S // KC
LAG = 2
TM = 512
NM = S // TM
NSPLIT = 4
TO = 128
NG = D // 128
HG = 128 // DH

OFF = 16
KM = KC - OFF

SAFE_BOUND = 80.0
QN_HI = 2.0 ** 40
KN_HI = 2.0 ** 60
V_HI = 2.0 ** 30
V_LO = 2.0 ** -20
K_TINY = 2.0 ** -50

F32 = jnp.float32
BF16 = jnp.bfloat16
NT = (((1,), (1,)), ((), ()))


def _ln(x):
    m = jnp.mean(x, axis=-1, keepdims=True)
    xc = x - m
    v = jnp.mean(xc * xc, axis=-1, keepdims=True)
    return xc * lax.rsqrt(v + EPS)


def _dot(a, b):
    return jnp.dot(a, b, preferred_element_type=F32)


def _dot_nt(a, b):
    return lax.dot_general(a, b, NT, preferred_element_type=F32)


def _kernel(x_hbm, wqkv_hbm, wo_hbm, w1t_hbm, w3t_hbm, w2_hbm, out_hbm,
            x_v, wqkv_v, wo_v, w1t_v, w3t_v, w2_v,
            xn_s, k_s, rt_s, qt_s, vt_s, ot_s, cs_s, cacc_s, va_s, qrow0_s, out_v, stat_s, flag_s,
            w_sems, x_sems, out_sems):
    def x_copy(b):
        return pltpu.make_async_copy(x_hbm.at[pl.ds(b * TM, TM), :],
                                     x_v.at[pl.ds(b * TM, TM), :], x_sems.at[b])

    def w_copy(j):
        return pltpu.make_async_copy(wqkv_hbm.at[:, pl.ds(j * D, D)],
                                     wqkv_v.at[:, pl.ds(j * D, D)], w_sems.at[j])

    cp_x = [x_copy(b) for b in range(NM)]
    cp_w = [w_copy(j) for j in range(3)]
    cp_rest = [pltpu.make_async_copy(src, dst, w_sems.at[3 + i])
               for i, (src, dst) in enumerate(((wo_hbm, wo_v), (w1t_hbm, w1t_v),
                                               (w3t_hbm, w3t_v), (w2_hbm, w2_v)))]

    et_rows = lax.broadcasted_iota(jnp.int32, (H, D), 0)
    et_cols = lax.broadcasted_iota(jnp.int32, (H, D), 1) // DH
    et = jnp.where(et_rows == et_cols, 1.0, 0.0).astype(BF16)

    def rows(b):
        return pl.ds(pl.multiple_of(b * TM, TM), TM)

    def ln1(b):
        xn_s[rows(b), :] = _ln(x_v[rows(b), :].astype(F32)).astype(BF16)

    def run_max(slot, nrow, val):
        m = stat_s[slot, 0:nrow, :]
        for j in range(TM // 128):
            m = jnp.maximum(m, val[:, j * 128:(j + 1) * 128])
        stat_s[slot, 0:nrow, :] = m

    def proj_k(b):
        k = _dot(xn_s[rows(b), :], wqkv_v[:, D:2 * D])
        kb = k.astype(BF16)
        half = pl.ds(pl.multiple_of(b * (TM // 2), TM // 2), TM // 2)
        lane = lax.broadcasted_iota(jnp.int32, (OFF, 128), 1)
        for g in range(NG):
            kg = kb[:, g * 128:(g + 1) * 128]
            k_s[g, half, :] = pltpu.bitcast(kg, jnp.uint32)
            for j in range(TM // KC):
                kk = kg[j * KC + KM:(j + 1) * KC, :].astype(F32)
                kk = jnp.where(jnp.abs(kk) < K_TINY, K_TINY, kk)
                ratio = kk / pltpu.roll(kk, 1, 1)
                r0 = pl.multiple_of((b * (TM // KC) + j) * OFF, OFF)
                rt_s[g, pl.ds(r0, OFF), :] = jnp.where(lane % DH == 0, kk, ratio)
        return (k * k).astype(BF16)

    def proj_q(b):
        qt = (_dot(xn_s[rows(b), :], wqkv_v[:, 0:D]) * QSCALE).T
        qt_s[b] = qt.astype(BF16)
        return (qt * qt).astype(BF16)

    def proj_v(b):
        vt = _dot(xn_s[rows(b), :], wqkv_v[:, 2 * D:3 * D]).T
        vt_s[b] = vt.astype(BF16)
        run_max(2, 8, jnp.abs(vt).reshape(D // 8, 8, TM).max(axis=0))

    def norm_k(ksq):
        run_max(0, H, _dot_nt(et, ksq))

    def norm_q(qsq):
        run_max(1, H, _dot(et, qsq))

    cp_x[0].start()
    cp_w[1].start()
    stat_s[...] = jnp.zeros(stat_s.shape, F32)
    cp_x[0].wait()
    cp_w[0].start()
    ln1(0)
    cp_w[1].wait()
    cp_w[2].start()
    cp_x[1].start()
    ksq0 = proj_k(0)
    cp_w[0].wait()
    cp_x[2].start()
    cp_x[3].start()
    qsq0 = proj_q(0)
    norm_k(ksq0)
    cp_w[2].wait()
    cp_x[1].wait()
    proj_v(0)
    norm_q(qsq0)
    ln1(1)
    cp_x[2].wait()
    cp_x[3].wait()
    for c in cp_rest:
        c.start()

    for b in range(1, NM):
        ksq = proj_k(b)
        qsq = proj_q(b)
        norm_k(ksq)
        proj_v(b)
        norm_q(qsq)
        if b + 1 < NM:
            ln1(b + 1)

    zeros16 = jnp.zeros((DH, TQ), BF16)

    def head_weights(qb, g, hh):
        qh = qt_s[qb, pl.ds(pl.multiple_of(g * 128 + hh * DH, DH), DH), :]
        return qh, jnp.concatenate([zeros16] * hh + [qh] + [zeros16] * (HG - 1 - hh), axis=0)

    def pv_step(s, row, c, acc, l):
        p = jnp.exp2(s)
        parts = [p[i * 8:(i + 1) * 8] for i in range(KC // 8)]
        m, v = parts[:KM // 8], parts[KM // 8:]
        for x in [v[0], m[0], v[1]] + m[1:]:
            l = l + x
        k0 = (c * KC) % TM
        vt = vt_s[(c * KC) // TM, pl.ds(row, DH), k0:k0 + KC]
        return acc + _dot(vt, p.astype(BF16)), l

    def finish(slot, hh, acc, l):
        lsum = l.sum(axis=0, keepdims=True)
        ot_s[slot, hh * DH:(hh + 1) * DH, :] = acc * (1.0 / lsum)

    def tail(it_prev, slot_prev, last):
        row = pl.multiple_of((it_prev % NG) * 128 + (HG - 1) * DH, DH)
        acc = cacc_s[0:DH, :]
        l = cacc_s[DH:DH + 8, :]
        for j in range(LAG):
            acc, l = pv_step(cs_s[j], row, NC - LAG + j, acc, l)
            last['acc'], last['l'] = acc, l
            yield None
        finish(slot_prev, HG - 1, acc, l)
        yield None

    def q_rows(qh):
        qf = qh.astype(F32)
        return [jnp.broadcast_to(qf[d:d + 1, :], (8, TQ)) for d in range(DH)]

    def vpu_scores(g, c, hh, qr):
        r = rt_s[g, c * OFF:(c + 1) * OFF, :]
        a = [qr[DH - 1]] * (OFF // 8)
        for d in range(DH - 1, -1, -1):
            rb = jnp.broadcast_to(r[:, hh * DH + d:hh * DH + d + 1], (OFF, TQ))
            a = [a[u] * rb[u * 8:(u + 1) * 8] for u in range(OFF // 8)]
            if d > 0:
                a = [x + qr[d - 1] for x in a]
        return a

    def precompute(it):
        row = pl.multiple_of((it % NG) * 128, 128)
        qr = q_rows(qt_s[it // NG, pl.ds(row, DH), :])
        a = vpu_scores(it % NG, 0, 0, qr)
        for u in range(OFF // 8):
            va_s[u * 8:(u + 1) * 8, :] = a[u]
        for d in range(DH):
            qrow0_s[d] = qr[d]

    def b_body(it, carry):
        qb = it // NG
        g = it % NG
        items = [(hh, c) for hh in range(HG) for c in range(NC)]
        n = len(items)
        w = {}
        qrow = {}
        acc = {}
        l = {}
        s = {}
        last = {}

        def qk(i):
            hh, c = items[i]
            if hh not in w:
                qh, w[hh] = head_weights(qb, g, hh)
                qrow[hh] = [qrow0_s[d] for d in range(DH)] if hh == 0 else q_rows(qh)
            p0 = c * (KC // 2)
            km = pltpu.bitcast(k_s[g, p0:p0 + KM // 2, :], BF16)
            sm = _dot(km, w[hh])
            if i == 0:
                a = [va_s[u * 8:(u + 1) * 8, :] for u in range(OFF // 8)]
            else:
                a = vpu_scores(g, c, hh, qrow[hh])
            sc = jnp.concatenate([sm] + a, axis=0)
            if i >= n - LAG:
                cs_s[i - (n - LAG)] = sc
            else:
                s[i] = sc

        def pv(i):
            hh, c = items[i]
            row = pl.multiple_of(g * 128 + hh * DH, DH)
            if c == 0:
                l[hh] = (l[hh - 1] if hh > 0 else last['l']) * 0.0
                acc[hh] = (acc[hh - 1] if hh > 0 else last['acc']) * 0.0
            acc[hh], l[hh] = pv_step(s.pop(i), row, c, acc[hh], l[hh])
            if c == NC - 1:
                finish(it, hh, acc[hh], l[hh])

        prev = tail(jnp.maximum(it - 1, 0), jnp.where(it == 0, NQ * NG, it - 1), last)
        for j in range(n):
            qk(j)
            if j >= LAG:
                pv(j - LAG)
            else:
                next(prev)
                if j == LAG - 1:
                    next(prev)
        cacc_s[0:DH, :] = acc[HG - 1]
        cacc_s[DH:DH + 8, :] = l[HG - 1]
        precompute(jnp.minimum(it + 1, NQ * NG - 1))
        return carry

    precompute(0)
    cs_s[...] = jnp.zeros(cs_s.shape, F32)
    cacc_s[...] = jnp.zeros(cacc_s.shape, F32)
    lax.fori_loop(0, NQ * NG, b_body, 0)
    for _ in tail(NQ * NG - 1, NQ * NG - 1, {}):
        pass

    bound2 = (jnp.max(stat_s[0], axis=1, keepdims=True)
              * jnp.max(stat_s[1], axis=1, keepdims=True))
    bound2 = jnp.max(bound2) * 1.05
    vm = jnp.max(stat_s[2, 0:8, :])
    safe = jnp.logical_and(bound2 <= SAFE_BOUND * SAFE_BOUND,
                           jnp.logical_and(vm <= V_HI, vm >= V_LO))
    safe = jnp.logical_and(safe, jnp.logical_and(jnp.max(stat_s[1]) <= QN_HI,
                                                 jnp.max(stat_s[0]) <= KN_HI))
    flag_s[0] = safe.astype(jnp.int32)

    @pl.when(flag_s[0] != 1)
    def _true_max_attention():
        head_rows = lax.broadcasted_iota(jnp.int32, (128, TQ), 0) // DH

        def body(it, carry):
            qb = it // H
            h = it % H
            g = h // HG
            hh = h % HG
            qg = qt_s[qb, pl.ds(pl.multiple_of(g * 128, 128), 128), :]
            w = jnp.where(head_rows == hh, qg, jnp.zeros_like(qg))
            row = pl.multiple_of(h * DH, DH)

            def scores(c):
                p0 = pl.multiple_of(c * (TM // 2), TM // 2)
                return _dot(pltpu.bitcast(k_s[g, pl.ds(p0, TM // 2), :], BF16), w)

            def max_pass(c, m):
                return jnp.maximum(m, jnp.max(scores(c), axis=0, keepdims=True))

            m = lax.fori_loop(0, NM, max_pass, jnp.full((1, TQ), -jnp.inf, F32))

            def sum_pass(c, al):
                acc, lsum = al
                p = jnp.exp2(scores(c) - m)
                return (acc + _dot(vt_s[c, pl.ds(row, DH), :], p.astype(BF16)),
                        lsum + jnp.sum(p, axis=0, keepdims=True))

            acc, lsum = lax.fori_loop(
                0, NM, sum_pass, (jnp.zeros((DH, TQ), F32), jnp.zeros((1, TQ), F32)))
            ot_s[qb * NG + g, pl.ds(pl.multiple_of(hh * DH, DH), DH), :] = acc * (1.0 / lsum)
            return carry

        lax.fori_loop(0, NQ * H, body, 0)

    for c in cp_rest:
        c.wait()

    def out_copy(b, j):
        r = pl.ds(pl.multiple_of(b * TM + j * TO, TO), TO)
        return pltpu.make_async_copy(out_v.at[r, :], out_hbm.at[r, :],
                                     out_sems.at[b * (TM // TO) + j])

    def c_body(b, carry):
        hs = []
        hns = []
        tr = TM // NSPLIT
        for j in range(NSPLIT):
            o = ot_s[pl.ds(b * NG, NG), :, j * tr:(j + 1) * tr].reshape(D, tr).T.astype(BF16)
            xr = x_v[pl.ds(pl.multiple_of(b * TM + j * tr, tr), tr), :].astype(F32)
            hj = xr + _dot(o, wo_v[...])
            hs.append(hj)
            hns.append(_ln(hj).astype(BF16))
        h = jnp.concatenate(hs, axis=0)
        hn = jnp.concatenate(hns, axis=0)
        gate = _dot_nt(hn, w1t_v[...])
        up = _dot_nt(hn, w3t_v[...])
        a = (gate * jax.nn.sigmoid(gate) * up).astype(BF16)
        for j in range(TM // TO):
            y = h[j * TO:(j + 1) * TO] + _dot(a[j * TO:(j + 1) * TO], w2_v[...])
            out_v[pl.ds(pl.multiple_of(b * TM + j * TO, TO), TO), :] = y.astype(BF16)
            out_copy(b, j).start()
        return carry

    lax.fori_loop(0, NM, c_body, 0)
    for b in range(NM):
        for j in range(TM // TO):
            out_copy(b, j).wait()


@jax.jit
def pallas_sequential_preLN__softmax_full_mha__glu_gated_swiglu__prompt_kernel(
    A_x: jax.Array,
    A_wqkv: jax.Array,
    A_wo: jax.Array,
    B_x: jax.Array,
    B_w1: jax.Array,
    B_w3: jax.Array,
    B_w2: jax.Array,
):
    del B_x
    x = A_x.reshape(S, D)
    hbm_spec = pl.BlockSpec(memory_space=pltpu.HBM)
    out = pl.pallas_call(
        _kernel,
        out_shape=jax.ShapeDtypeStruct((S, D), BF16),
        in_specs=[hbm_spec] * 6,
        out_specs=hbm_spec,
        scratch_shapes=[
            pltpu.VMEM((S, D), BF16),
            pltpu.VMEM((D, 3 * D), BF16),
            pltpu.VMEM((D, D), BF16),
            pltpu.VMEM((F, D), BF16),
            pltpu.VMEM((F, D), BF16),
            pltpu.VMEM((F, D), BF16),
            pltpu.VMEM((S, D), BF16),
            pltpu.VMEM((NG, S // 2, 128), jnp.uint32),
            pltpu.VMEM((NG, NC * OFF, 128), F32),
            pltpu.VMEM((NQ, D, TQ), BF16),
            pltpu.VMEM((NM, D, TM), BF16),
            pltpu.VMEM((NQ * NG + 1, 128, TQ), F32),
            pltpu.VMEM((LAG, KC, TQ), F32),
            pltpu.VMEM((DH + 8, TQ), F32),
            pltpu.VMEM((OFF, TQ), F32),
            pltpu.VMEM((DH, 8, TQ), F32),
            pltpu.VMEM((S, D), BF16),
            pltpu.VMEM((3, H, 128), F32),
            pltpu.SMEM((1,), jnp.int32),
            pltpu.SemaphoreType.DMA((7,)),
            pltpu.SemaphoreType.DMA((NM,)),
            pltpu.SemaphoreType.DMA((S // TO,)),
        ],
        compiler_params=pltpu.CompilerParams(vmem_limit_bytes=100 * 1024 * 1024),
        name="preln_mha_swiglu",
    )(x, A_wqkv, A_wo, B_w1.T, B_w3.T, B_w2)
    return out.reshape(1, S, D)
```

```python
import jax
import jax.numpy as jnp
from jax import lax
import jax.experimental.pallas as pl
import jax.experimental.pallas.tpu as pltpu

S = 2048
D = 512
H = 32
DH = 16
F = 1376
EPS = 1e-5
LOG2E = 1.4426950408889634
QSCALE = (DH ** -0.5) * LOG2E

TQ = 512
NQ = S // TQ
KC = 128
NC = S // KC
LAG = 2
TM = 512
NM = S // TM
NSPLIT = 4
TO = 128
NG = D // 128
HG = 128 // DH

OFF = 16
KM = KC - OFF

SAFE_BOUND = 80.0
QN_HI = 2.0 ** 40
KN_HI = 2.0 ** 60
V_HI = 2.0 ** 30
V_LO = 2.0 ** -20
K_TINY = 2.0 ** -50

F32 = jnp.float32
BF16 = jnp.bfloat16
NT = (((1,), (1,)), ((), ()))


def _ln(x):
    m = jnp.mean(x, axis=-1, keepdims=True)
    xc = x - m
    v = jnp.mean(xc * xc, axis=-1, keepdims=True)
    return xc * lax.rsqrt(v + EPS)


def _dot(a, b):
    return jnp.dot(a, b, preferred_element_type=F32)


def _dot_nt(a, b):
    return lax.dot_general(a, b, NT, preferred_element_type=F32)


def _kernel(x_hbm, wqkv_hbm, wo_hbm, w1t_hbm, w3t_hbm, w2_hbm, out_hbm,
            x_v, wqkv_v, wo_v, w1t_v, w3t_v, w2_v,
            xn_s, k_s, rt_s, qt_s, vt_s, ot_s, cs_s, cacc_s, va_s, qrow0_s, o0_s, out_v, stat_s, flag_s,
            w_sems, x_sems, out_sems):
    def x_copy(b):
        return pltpu.make_async_copy(x_hbm.at[pl.ds(b * TM, TM), :],
                                     x_v.at[pl.ds(b * TM, TM), :], x_sems.at[b])

    def w_copy(j):
        return pltpu.make_async_copy(wqkv_hbm.at[:, pl.ds(j * D, D)],
                                     wqkv_v.at[:, pl.ds(j * D, D)], w_sems.at[j])

    cp_x = [x_copy(b) for b in range(NM)]
    cp_w = [w_copy(j) for j in range(3)]
    cp_rest = [pltpu.make_async_copy(src, dst, w_sems.at[3 + i])
               for i, (src, dst) in enumerate(((wo_hbm, wo_v), (w1t_hbm, w1t_v),
                                               (w3t_hbm, w3t_v), (w2_hbm, w2_v)))]

    et_rows = lax.broadcasted_iota(jnp.int32, (H, D), 0)
    et_cols = lax.broadcasted_iota(jnp.int32, (H, D), 1) // DH
    et = jnp.where(et_rows == et_cols, 1.0, 0.0).astype(BF16)

    def rows(b):
        return pl.ds(pl.multiple_of(b * TM, TM), TM)

    def ln1(b):
        xn_s[rows(b), :] = _ln(x_v[rows(b), :].astype(F32)).astype(BF16)

    def run_max(slot, nrow, val):
        m = stat_s[slot, 0:nrow, :]
        for j in range(TM // 128):
            m = jnp.maximum(m, val[:, j * 128:(j + 1) * 128])
        stat_s[slot, 0:nrow, :] = m

    def proj_k(b):
        k = _dot(xn_s[rows(b), :], wqkv_v[:, D:2 * D])
        kb = k.astype(BF16)
        half = pl.ds(pl.multiple_of(b * (TM // 2), TM // 2), TM // 2)
        lane = lax.broadcasted_iota(jnp.int32, (OFF, 128), 1)
        for g in range(NG):
            kg = kb[:, g * 128:(g + 1) * 128]
            k_s[g, half, :] = pltpu.bitcast(kg, jnp.uint32)
            for j in range(TM // KC):
                kk = kg[j * KC + KM:(j + 1) * KC, :].astype(F32)
                kk = jnp.where(jnp.abs(kk) < K_TINY, K_TINY, kk)
                ratio = kk / pltpu.roll(kk, 1, 1)
                r0 = pl.multiple_of((b * (TM // KC) + j) * OFF, OFF)
                rt_s[g, pl.ds(r0, OFF), :] = jnp.where(lane % DH == 0, kk, ratio)
        return (k * k).astype(BF16)

    def proj_q(b):
        qt = (_dot(xn_s[rows(b), :], wqkv_v[:, 0:D]) * QSCALE).T
        qt_s[b] = qt.astype(BF16)
        return (qt * qt).astype(BF16)

    def proj_v(b):
        vt = _dot(xn_s[rows(b), :], wqkv_v[:, 2 * D:3 * D]).T
        vt_s[b] = vt.astype(BF16)
        run_max(2, 8, jnp.abs(vt).reshape(D // 8, 8, TM).max(axis=0))

    def norm_k(ksq):
        run_max(0, H, _dot_nt(et, ksq))

    def norm_q(qsq):
        run_max(1, H, _dot(et, qsq))

    cp_x[0].start()
    cp_w[1].start()
    stat_s[...] = jnp.zeros(stat_s.shape, F32)
    cp_x[0].wait()
    cp_w[0].start()
    ln1(0)
    cp_w[1].wait()
    cp_w[2].start()
    cp_x[1].start()
    ksq0 = proj_k(0)
    cp_w[0].wait()
    cp_x[2].start()
    cp_x[3].start()
    qsq0 = proj_q(0)
    norm_k(ksq0)
    cp_w[2].wait()
    cp_x[1].wait()
    proj_v(0)
    norm_q(qsq0)
    ln1(1)
    cp_x[2].wait()
    cp_x[3].wait()
    for c in cp_rest:
        c.start()

    for b in range(1, NM):
        ksq = proj_k(b)
        qsq = proj_q(b)
        norm_k(ksq)
        proj_v(b)
        norm_q(qsq)
        if b + 1 < NM:
            ln1(b + 1)

    zeros16 = jnp.zeros((DH, TQ), BF16)

    def head_weights(qb, g, hh):
        qh = qt_s[qb, pl.ds(pl.multiple_of(g * 128 + hh * DH, DH), DH), :]
        return qh, jnp.concatenate([zeros16] * hh + [qh] + [zeros16] * (HG - 1 - hh), axis=0)

    def pv_step(s, row, c, acc, l):
        p = jnp.exp2(s)
        parts = [p[i * 8:(i + 1) * 8] for i in range(KC // 8)]
        m, v = parts[:KM // 8], parts[KM // 8:]
        for x in [v[0], m[0], v[1]] + m[1:]:
            l = l + x
        k0 = (c * KC) % TM
        vt = vt_s[(c * KC) // TM, pl.ds(row, DH), k0:k0 + KC]
        return acc + _dot(vt, p.astype(BF16)), l

    def finish(slot, hh, acc, l):
        lsum = l.sum(axis=0, keepdims=True)
        ot_s[slot, hh * DH:(hh + 1) * DH, :] = acc * (1.0 / lsum)

    def tail(it_prev, slot_prev, last):
        row = pl.multiple_of((it_prev % NG) * 128 + (HG - 1) * DH, DH)
        acc = cacc_s[0:DH, :]
        l = cacc_s[DH:DH + 8, :]
        for j in range(LAG):
            acc, l = pv_step(cs_s[j], row, NC - LAG + j, acc, l)
            last['acc'], last['l'] = acc, l
            yield None
        finish(slot_prev, HG - 1, acc, l)
        yield None

    def q_rows(qh):
        qf = qh.astype(F32)
        return [jnp.broadcast_to(qf[d:d + 1, :], (8, TQ)) for d in range(DH)]

    def vpu_scores(g, c, hh, qr):
        r = rt_s[g, c * OFF:(c + 1) * OFF, :]
        a = [qr[DH - 1]] * (OFF // 8)
        for d in range(DH - 1, -1, -1):
            rb = jnp.broadcast_to(r[:, hh * DH + d:hh * DH + d + 1], (OFF, TQ))
            a = [a[u] * rb[u * 8:(u + 1) * 8] for u in range(OFF // 8)]
            if d > 0:
                a = [x + qr[d - 1] for x in a]
        return a

    def precompute(it):
        row = pl.multiple_of((it % NG) * 128, 128)
        qr = q_rows(qt_s[it // NG, pl.ds(row, DH), :])
        a = vpu_scores(it % NG, 0, 0, qr)
        for u in range(OFF // 8):
            va_s[u * 8:(u + 1) * 8, :] = a[u]
        for d in range(DH):
            qrow0_s[d] = qr[d]

    def b_body(it, carry):
        qb = it // NG
        g = it % NG
        items = [(hh, c) for hh in range(HG) for c in range(NC)]
        n = len(items)
        w = {}
        qrow = {}
        acc = {}
        l = {}
        s = {}
        last = {}

        def qk(i):
            hh, c = items[i]
            if hh not in w:
                qh, w[hh] = head_weights(qb, g, hh)
                qrow[hh] = [qrow0_s[d] for d in range(DH)] if hh == 0 else q_rows(qh)
            p0 = c * (KC // 2)
            km = pltpu.bitcast(k_s[g, p0:p0 + KM // 2, :], BF16)
            sm = _dot(km, w[hh])
            if i == 0:
                a = [va_s[u * 8:(u + 1) * 8, :] for u in range(OFF // 8)]
            else:
                a = vpu_scores(g, c, hh, qrow[hh])
            sc = jnp.concatenate([sm] + a, axis=0)
            if i >= n - LAG:
                cs_s[i - (n - LAG)] = sc
            else:
                s[i] = sc

        def pv(i):
            hh, c = items[i]
            row = pl.multiple_of(g * 128 + hh * DH, DH)
            if c == 0:
                l[hh] = (l[hh - 1] if hh > 0 else last['l']) * 0.0
                acc[hh] = (acc[hh - 1] if hh > 0 else last['acc']) * 0.0
            acc[hh], l[hh] = pv_step(s.pop(i), row, c, acc[hh], l[hh])
            if c == NC - 1:
                finish(it, hh, acc[hh], l[hh])

        prev = tail(jnp.maximum(it - 1, 0), jnp.where(it == 0, NQ * NG, it - 1), last)
        for j in range(n):
            qk(j)
            if j >= LAG:
                pv(j - LAG)
            else:
                next(prev)
                if j == LAG - 1:
                    next(prev)
        cacc_s[0:DH, :] = acc[HG - 1]
        cacc_s[DH:DH + 8, :] = l[HG - 1]
        precompute(jnp.minimum(it + 1, NQ * NG - 1))
        return carry

    precompute(0)
    cs_s[...] = jnp.zeros(cs_s.shape, F32)
    cacc_s[...] = jnp.zeros(cacc_s.shape, F32)
    lax.fori_loop(0, NQ * NG, b_body, 0)
    for _ in tail(NQ * NG - 1, NQ * NG - 1, {}):
        pass

    tr = TM // NSPLIT

    def o_piece(b, j):
        return ot_s[pl.ds(b * NG, NG), :, j * tr:(j + 1) * tr].reshape(D, tr).T.astype(BF16)

    o0_s[...] = o_piece(0, 0)

    bound2 = (jnp.max(stat_s[0], axis=1, keepdims=True)
              * jnp.max(stat_s[1], axis=1, keepdims=True))
    bound2 = jnp.max(bound2) * 1.05
    vm = jnp.max(stat_s[2, 0:8, :])
    safe = jnp.logical_and(bound2 <= SAFE_BOUND * SAFE_BOUND,
                           jnp.logical_and(vm <= V_HI, vm >= V_LO))
    safe = jnp.logical_and(safe, jnp.logical_and(jnp.max(stat_s[1]) <= QN_HI,
                                                 jnp.max(stat_s[0]) <= KN_HI))
    flag_s[0] = safe.astype(jnp.int32)

    @pl.when(flag_s[0] != 1)
    def _true_max_attention():
        head_rows = lax.broadcasted_iota(jnp.int32, (128, TQ), 0) // DH

        def body(it, carry):
            qb = it // H
            h = it % H
            g = h // HG
            hh = h % HG
            qg = qt_s[qb, pl.ds(pl.multiple_of(g * 128, 128), 128), :]
            w = jnp.where(head_rows == hh, qg, jnp.zeros_like(qg))
            row = pl.multiple_of(h * DH, DH)

            def scores(c):
                p0 = pl.multiple_of(c * (TM // 2), TM // 2)
                return _dot(pltpu.bitcast(k_s[g, pl.ds(p0, TM // 2), :], BF16), w)

            def max_pass(c, m):
                return jnp.maximum(m, jnp.max(scores(c), axis=0, keepdims=True))

            m = lax.fori_loop(0, NM, max_pass, jnp.full((1, TQ), -jnp.inf, F32))

            def sum_pass(c, al):
                acc, lsum = al
                p = jnp.exp2(scores(c) - m)
                return (acc + _dot(vt_s[c, pl.ds(row, DH), :], p.astype(BF16)),
                        lsum + jnp.sum(p, axis=0, keepdims=True))

            acc, lsum = lax.fori_loop(
                0, NM, sum_pass, (jnp.zeros((DH, TQ), F32), jnp.zeros((1, TQ), F32)))
            ot_s[qb * NG + g, pl.ds(pl.multiple_of(hh * DH, DH), DH), :] = acc * (1.0 / lsum)
            return carry

        lax.fori_loop(0, NQ * H, body, 0)
        o0_s[...] = o_piece(0, 0)

    for c in cp_rest:
        c.wait()

    def out_copy(b, j):
        r = pl.ds(pl.multiple_of(b * TM + j * TO, TO), TO)
        return pltpu.make_async_copy(out_v.at[r, :], out_hbm.at[r, :],
                                     out_sems.at[b * (TM // TO) + j])

    def c_body(b, carry):
        hs = []
        hns = []
        for j in range(NSPLIT):
            o = o0_s[...] if j == 0 else o_piece(b, j)
            xr = x_v[pl.ds(pl.multiple_of(b * TM + j * tr, tr), tr), :].astype(F32)
            hj = xr + _dot(o, wo_v[...])
            hs.append(hj)
            hns.append(_ln(hj).astype(BF16))
        h = jnp.concatenate(hs, axis=0)
        hn = jnp.concatenate(hns, axis=0)
        gate = _dot_nt(hn, w1t_v[...])
        up = _dot_nt(hn, w3t_v[...])
        a = (gate * jax.nn.sigmoid(gate) * up).astype(BF16)
        for j in range(TM // TO):
            y = h[j * TO:(j + 1) * TO] + _dot(a[j * TO:(j + 1) * TO], w2_v[...])
            out_v[pl.ds(pl.multiple_of(b * TM + j * TO, TO), TO), :] = y.astype(BF16)
            out_copy(b, j).start()
        o0_s[...] = o_piece(jnp.minimum(b + 1, NM - 1), 0)
        return carry

    lax.fori_loop(0, NM, c_body, 0)
    for b in range(NM):
        for j in range(TM // TO):
            out_copy(b, j).wait()


@jax.jit
def pallas_sequential_preLN__softmax_full_mha__glu_gated_swiglu__prompt_kernel(
    A_x: jax.Array,
    A_wqkv: jax.Array,
    A_wo: jax.Array,
    B_x: jax.Array,
    B_w1: jax.Array,
    B_w3: jax.Array,
    B_w2: jax.Array,
):
    del B_x
    x = A_x.reshape(S, D)
    hbm_spec = pl.BlockSpec(memory_space=pltpu.HBM)
    out = pl.pallas_call(
        _kernel,
        out_shape=jax.ShapeDtypeStruct((S, D), BF16),
        in_specs=[hbm_spec] * 6,
        out_specs=hbm_spec,
        scratch_shapes=[
            pltpu.VMEM((S, D), BF16),
            pltpu.VMEM((D, 3 * D), BF16),
            pltpu.VMEM((D, D), BF16),
            pltpu.VMEM((F, D), BF16),
            pltpu.VMEM((F, D), BF16),
            pltpu.VMEM((F, D), BF16),
            pltpu.VMEM((S, D), BF16),
            pltpu.VMEM((NG, S // 2, 128), jnp.uint32),
            pltpu.VMEM((NG, NC * OFF, 128), F32),
            pltpu.VMEM((NQ, D, TQ), BF16),
            pltpu.VMEM((NM, D, TM), BF16),
            pltpu.VMEM((NQ * NG + 1, 128, TQ), F32),
            pltpu.VMEM((LAG, KC, TQ), F32),
            pltpu.VMEM((DH + 8, TQ), F32),
            pltpu.VMEM((OFF, TQ), F32),
            pltpu.VMEM((DH, 8, TQ), F32),
            pltpu.VMEM((TM // NSPLIT, D), BF16),
            pltpu.VMEM((S, D), BF16),
            pltpu.VMEM((3, H, 128), F32),
            pltpu.SMEM((1,), jnp.int32),
            pltpu.SemaphoreType.DMA((7,)),
            pltpu.SemaphoreType.DMA((NM,)),
            pltpu.SemaphoreType.DMA((S // TO,)),
        ],
        compiler_params=pltpu.CompilerParams(vmem_limit_bytes=100 * 1024 * 1024),
        name="preln_mha_swiglu",
    )(x, A_wqkv, A_wo, B_w1.T, B_w3.T, B_w2)
    return out.reshape(1, S, D)
```

```python
import jax
import jax.numpy as jnp
from jax import lax
import jax.experimental.pallas as pl
import jax.experimental.pallas.tpu as pltpu

S = 2048
D = 512
H = 32
DH = 16
F = 1376
EPS = 1e-5
LOG2E = 1.4426950408889634
QSCALE = (DH ** -0.5) * LOG2E

TQ = 512
NQ = S // TQ
KC = 128
NC = S // KC
LAG = 2
TM = 512
NM = S // TM
NSPLIT = 4
TO = 128
NG = D // 128
HG = 128 // DH

OFF = 16
KM = KC - OFF

SAFE_BOUND = 80.0
QN_HI = 2.0 ** 40
KN_HI = 2.0 ** 60
V_HI = 2.0 ** 30
V_LO = 2.0 ** -20
K_TINY = 2.0 ** -50

F32 = jnp.float32
BF16 = jnp.bfloat16
NT = (((1,), (1,)), ((), ()))


def _ln(x):
    m = jnp.mean(x, axis=-1, keepdims=True)
    xc = x - m
    v = jnp.mean(xc * xc, axis=-1, keepdims=True)
    return xc * lax.rsqrt(v + EPS)


def _dot(a, b):
    return jnp.dot(a, b, preferred_element_type=F32)


def _dot_nt(a, b):
    return lax.dot_general(a, b, NT, preferred_element_type=F32)


def _kernel(x_hbm, wqkv_hbm, wo_hbm, w1t_hbm, w3t_hbm, w2_hbm, out_hbm,
            x_v, wqkv_v, wo_v, w1t_v, w3t_v, w2_v,
            xn_s, k_s, rt_s, qt_s, vt_s, ot_s, cs_s, cp_s, cacc_s, va_s, qrow0_s, o0_s, out_v, stat_s, kmax_s, flag_s,
            w_sems, x_sems, out_sems):
    def x_copy(b):
        return pltpu.make_async_copy(x_hbm.at[pl.ds(b * TM, TM), :],
                                     x_v.at[pl.ds(b * TM, TM), :], x_sems.at[b])

    def w_copy(j):
        return pltpu.make_async_copy(wqkv_hbm.at[:, pl.ds(j * D, D)],
                                     wqkv_v.at[:, pl.ds(j * D, D)], w_sems.at[j])

    cp_x = [x_copy(b) for b in range(NM)]
    cp_w = [w_copy(j) for j in range(3)]
    cp_rest = [pltpu.make_async_copy(src, dst, w_sems.at[3 + i])
               for i, (src, dst) in enumerate(((wo_hbm, wo_v), (w1t_hbm, w1t_v),
                                               (w3t_hbm, w3t_v), (w2_hbm, w2_v)))]

    et_rows = lax.broadcasted_iota(jnp.int32, (H, D), 0)
    et_cols = lax.broadcasted_iota(jnp.int32, (H, D), 1) // DH
    et = jnp.where(et_rows == et_cols, 1.0, 0.0).astype(BF16)

    def rows(b):
        return pl.ds(pl.multiple_of(b * TM, TM), TM)

    def ln1(b):
        xn_s[rows(b), :] = _ln(x_v[rows(b), :].astype(F32)).astype(BF16)

    def run_max(slot, nrow, val):
        m = stat_s[slot, 0:nrow, :]
        for j in range(TM // 128):
            m = jnp.maximum(m, val[:, j * 128:(j + 1) * 128])
        stat_s[slot, 0:nrow, :] = m

    def proj_k(b):
        k = _dot(xn_s[rows(b), :], wqkv_v[:, D:2 * D])
        kb = k.astype(BF16)
        half = pl.ds(pl.multiple_of(b * (TM // 2), TM // 2), TM // 2)
        lane = lax.broadcasted_iota(jnp.int32, (OFF, 128), 1)
        for g in range(NG):
            kg = kb[:, g * 128:(g + 1) * 128]
            k_s[g, half, :] = pltpu.bitcast(kg, jnp.uint32)
            for j in range(TM // KC):
                kk = kg[j * KC + KM:(j + 1) * KC, :].astype(F32)
                kk = jnp.where(jnp.abs(kk) < K_TINY, K_TINY, kk)
                ratio = kk / pltpu.roll(kk, 1, 1)
                r0 = pl.multiple_of((b * (TM // KC) + j) * OFF, OFF)
                rt_s[g, pl.ds(r0, OFF), :] = jnp.where(lane % DH == 0, kk, ratio)
        kmax_s[...] = jnp.maximum(kmax_s[...], jnp.abs(k).reshape(TM // 8, 8, D).max(axis=0))

    def proj_q(b):
        qt = (_dot(xn_s[rows(b), :], wqkv_v[:, 0:D]) * QSCALE).T
        qt_s[b] = qt.astype(BF16)
        return (qt * qt).astype(BF16)

    def proj_v(b):
        vt = _dot(xn_s[rows(b), :], wqkv_v[:, 2 * D:3 * D]).T
        vt_s[b] = vt.astype(BF16)
        run_max(2, 8, jnp.abs(vt).reshape(D // 8, 8, TM).max(axis=0))

    def norm_q(qsq):
        run_max(1, H, _dot(et, qsq))

    cp_x[0].start()
    cp_w[1].start()
    stat_s[...] = jnp.zeros(stat_s.shape, F32)
    kmax_s[...] = jnp.zeros(kmax_s.shape, F32)
    cp_x[0].wait()
    cp_w[0].start()
    ln1(0)
    cp_w[1].wait()
    cp_w[2].start()
    cp_x[1].start()
    proj_k(0)
    cp_w[0].wait()
    cp_x[2].start()
    cp_x[3].start()
    qsq0 = proj_q(0)
    cp_w[2].wait()
    cp_x[1].wait()
    proj_v(0)
    norm_q(qsq0)
    ln1(1)
    cp_x[2].wait()
    cp_x[3].wait()
    for c in cp_rest:
        c.start()

    for b in range(1, NM):
        proj_k(b)
        qsq = proj_q(b)
        proj_v(b)
        norm_q(qsq)
        if b + 1 < NM:
            ln1(b + 1)

    zeros16 = jnp.zeros((DH, TQ), BF16)

    def head_weights(qb, g, hh):
        qh = qt_s[qb, pl.ds(pl.multiple_of(g * 128 + hh * DH, DH), DH), :]
        return qh, jnp.concatenate([zeros16] * hh + [qh] + [zeros16] * (HG - 1 - hh), axis=0)

    def probs(s, l):
        p = jnp.exp2(s)
        parts = [p[i * 8:(i + 1) * 8] for i in range(KC // 8)]
        m, v = parts[:KM // 8], parts[KM // 8:]
        for x in [v[0], m[0], v[1]] + m[1:]:
            l = l + x
        return p.astype(BF16), l

    def pv_dot(pb, row, c, acc):
        k0 = (c * KC) % TM
        vt = vt_s[(c * KC) // TM, pl.ds(row, DH), k0:k0 + KC]
        return acc + _dot(vt, pb)

    def pv_step(s, row, c, acc, l):
        pb, l = probs(s, l)
        return pv_dot(pb, row, c, acc), l

    def finish(slot, hh, acc, l):
        lsum = l.sum(axis=0, keepdims=True)
        ot_s[slot, hh * DH:(hh + 1) * DH, :] = acc * (1.0 / lsum)

    def tail(it_prev, slot_prev, last):
        row = pl.multiple_of((it_prev % NG) * 128 + (HG - 1) * DH, DH)
        acc = cacc_s[0:DH, :]
        l = cacc_s[DH:DH + 8, :]
        acc = pv_dot(pltpu.bitcast(cp_s[...], BF16), row, NC - 2, acc)
        last['acc'], last['l'] = acc, l
        yield None
        acc, l = pv_step(cs_s[...], row, NC - 1, acc, l)
        last['acc'], last['l'] = acc, l
        yield None
        finish(slot_prev, HG - 1, acc, l)
        yield None

    def q_rows(qh):
        qf = qh.astype(F32)
        return [jnp.broadcast_to(qf[d:d + 1, :], (8, TQ)) for d in range(DH)]

    def vpu_scores(g, c, hh, qr):
        r = rt_s[g, c * OFF:(c + 1) * OFF, :]
        a = [qr[DH - 1]] * (OFF // 8)
        for d in range(DH - 1, -1, -1):
            rb = jnp.broadcast_to(r[:, hh * DH + d:hh * DH + d + 1], (OFF, TQ))
            a = [a[u] * rb[u * 8:(u + 1) * 8] for u in range(OFF // 8)]
            if d > 0:
                a = [x + qr[d - 1] for x in a]
        return a

    def precompute(it):
        row = pl.multiple_of((it % NG) * 128, 128)
        qr = q_rows(qt_s[it // NG, pl.ds(row, DH), :])
        a = vpu_scores(it % NG, 0, 0, qr)
        for u in range(OFF // 8):
            va_s[u * 8:(u + 1) * 8, :] = a[u]
        for d in range(DH):
            qrow0_s[d] = qr[d]

    def b_body(it, carry):
        qb = it // NG
        g = it % NG
        items = [(hh, c) for hh in range(HG) for c in range(NC)]
        n = len(items)
        w = {}
        qrow = {}
        acc = {}
        l = {}
        s = {}
        last = {}

        def qk(i):
            hh, c = items[i]
            if hh not in w:
                qh, w[hh] = head_weights(qb, g, hh)
                qrow[hh] = [qrow0_s[d] for d in range(DH)] if hh == 0 else q_rows(qh)
            p0 = c * (KC // 2)
            km = pltpu.bitcast(k_s[g, p0:p0 + KM // 2, :], BF16)
            sm = _dot(km, w[hh])
            if i == 0:
                a = [va_s[u * 8:(u + 1) * 8, :] for u in range(OFF // 8)]
            else:
                a = vpu_scores(g, c, hh, qrow[hh])
            sc = jnp.concatenate([sm] + a, axis=0)
            if i == n - 1:
                cs_s[...] = sc
            else:
                s[i] = sc

        def pv(i):
            hh, c = items[i]
            row = pl.multiple_of(g * 128 + hh * DH, DH)
            if c == 0:
                l[hh] = (l[hh - 1] if hh > 0 else last['l']) * 0.0
                acc[hh] = (acc[hh - 1] if hh > 0 else last['acc']) * 0.0
            acc[hh], l[hh] = pv_step(s.pop(i), row, c, acc[hh], l[hh])
            if c == NC - 1:
                finish(it, hh, acc[hh], l[hh])

        prev = tail(jnp.maximum(it - 1, 0), jnp.where(it == 0, NQ * NG, it - 1), last)
        for j in range(n):
            qk(j)
            if j >= LAG:
                pv(j - LAG)
            else:
                next(prev)
                if j == LAG - 1:
                    next(prev)
        pb, l_last = probs(s.pop(n - 2), l[HG - 1])
        cp_s[...] = pltpu.bitcast(pb, jnp.uint32)
        cacc_s[0:DH, :] = acc[HG - 1]
        cacc_s[DH:DH + 8, :] = l_last
        precompute(jnp.minimum(it + 1, NQ * NG - 1))
        return carry

    precompute(0)
    cs_s[...] = jnp.zeros(cs_s.shape, F32)
    cp_s[...] = jnp.zeros(cp_s.shape, jnp.uint32)
    cacc_s[...] = jnp.zeros(cacc_s.shape, F32)
    lax.fori_loop(0, NQ * NG, b_body, 0)
    for _ in tail(NQ * NG - 1, NQ * NG - 1, {}):
        pass

    tr = TM // NSPLIT

    def o_piece(b, j):
        return ot_s[pl.ds(b * NG, NG), :, j * tr:(j + 1) * tr].reshape(D, tr).T.astype(BF16)

    o0_s[...] = o_piece(0, 0)

    kcol = jnp.max(kmax_s[...], axis=0, keepdims=True)
    kn = jnp.sum(jnp.where(et_rows == et_cols, kcol * kcol, 0.0), axis=1, keepdims=True)
    bound2 = kn * jnp.max(stat_s[1], axis=1, keepdims=True)
    bound2 = jnp.max(bound2) * 1.05
    vm = jnp.max(stat_s[2, 0:8, :])
    safe = jnp.logical_and(bound2 <= SAFE_BOUND * SAFE_BOUND,
                           jnp.logical_and(vm <= V_HI, vm >= V_LO))
    safe = jnp.logical_and(safe, jnp.logical_and(jnp.max(stat_s[1]) <= QN_HI,
                                                 jnp.max(kn) <= KN_HI))
    flag_s[0] = safe.astype(jnp.int32)

    @pl.when(flag_s[0] != 1)
    def _true_max_attention():
        head_rows = lax.broadcasted_iota(jnp.int32, (128, TQ), 0) // DH

        def body(it, carry):
            qb = it // H
            h = it % H
            g = h // HG
            hh = h % HG
            qg = qt_s[qb, pl.ds(pl.multiple_of(g * 128, 128), 128), :]
            w = jnp.where(head_rows == hh, qg, jnp.zeros_like(qg))
            row = pl.multiple_of(h * DH, DH)

            def scores(c):
                p0 = pl.multiple_of(c * (TM // 2), TM // 2)
                return _dot(pltpu.bitcast(k_s[g, pl.ds(p0, TM // 2), :], BF16), w)

            def max_pass(c, m):
                return jnp.maximum(m, jnp.max(scores(c), axis=0, keepdims=True))

            m = lax.fori_loop(0, NM, max_pass, jnp.full((1, TQ), -jnp.inf, F32))

            def sum_pass(c, al):
                acc, lsum = al
                p = jnp.exp2(scores(c) - m)
                return (acc + _dot(vt_s[c, pl.ds(row, DH), :], p.astype(BF16)),
                        lsum + jnp.sum(p, axis=0, keepdims=True))

            acc, lsum = lax.fori_loop(
                0, NM, sum_pass, (jnp.zeros((DH, TQ), F32), jnp.zeros((1, TQ), F32)))
            ot_s[qb * NG + g, pl.ds(pl.multiple_of(hh * DH, DH), DH), :] = acc * (1.0 / lsum)
            return carry

        lax.fori_loop(0, NQ * H, body, 0)
        o0_s[...] = o_piece(0, 0)

    for c in cp_rest:
        c.wait()

    def out_copy(b, j):
        r = pl.ds(pl.multiple_of(b * TM + j * TO, TO), TO)
        return pltpu.make_async_copy(out_v.at[r, :], out_hbm.at[r, :],
                                     out_sems.at[b * (TM // TO) + j])

    def c_body(b, carry):
        hs = []
        hns = []
        for j in range(NSPLIT):
            o = o0_s[...] if j == 0 else o_piece(b, j)
            xr = x_v[pl.ds(pl.multiple_of(b * TM + j * tr, tr), tr), :].astype(F32)
            hj = xr + _dot(o, wo_v[...])
            hs.append(hj)
            hns.append(_ln(hj).astype(BF16))
        h = jnp.concatenate(hs, axis=0)
        hn = jnp.concatenate(hns, axis=0)
        gate = _dot_nt(hn, w1t_v[...])
        up = _dot_nt(hn, w3t_v[...])
        a = (gate * jax.nn.sigmoid(gate) * up).astype(BF16)
        for j in range(TM // TO):
            y = h[j * TO:(j + 1) * TO] + _dot(a[j * TO:(j + 1) * TO], w2_v[...])
            out_v[pl.ds(pl.multiple_of(b * TM + j * TO, TO), TO), :] = y.astype(BF16)
            out_copy(b, j).start()
        o0_s[...] = o_piece(jnp.minimum(b + 1, NM - 1), 0)
        return carry

    lax.fori_loop(0, NM, c_body, 0)
    for b in range(NM):
        for j in range(TM // TO):
            out_copy(b, j).wait()


@jax.jit
def pallas_sequential_preLN__softmax_full_mha__glu_gated_swiglu__prompt_kernel(
    A_x: jax.Array,
    A_wqkv: jax.Array,
    A_wo: jax.Array,
    B_x: jax.Array,
    B_w1: jax.Array,
    B_w3: jax.Array,
    B_w2: jax.Array,
):
    del B_x
    x = A_x.reshape(S, D)
    hbm_spec = pl.BlockSpec(memory_space=pltpu.HBM)
    out = pl.pallas_call(
        _kernel,
        out_shape=jax.ShapeDtypeStruct((S, D), BF16),
        in_specs=[hbm_spec] * 6,
        out_specs=hbm_spec,
        scratch_shapes=[
            pltpu.VMEM((S, D), BF16),
            pltpu.VMEM((D, 3 * D), BF16),
            pltpu.VMEM((D, D), BF16),
            pltpu.VMEM((F, D), BF16),
            pltpu.VMEM((F, D), BF16),
            pltpu.VMEM((F, D), BF16),
            pltpu.VMEM((S, D), BF16),
            pltpu.VMEM((NG, S // 2, 128), jnp.uint32),
            pltpu.VMEM((NG, NC * OFF, 128), F32),
            pltpu.VMEM((NQ, D, TQ), BF16),
            pltpu.VMEM((NM, D, TM), BF16),
            pltpu.VMEM((NQ * NG + 1, 128, TQ), F32),
            pltpu.VMEM((KC, TQ), F32),
            pltpu.VMEM((KC // 2, TQ), jnp.uint32),
            pltpu.VMEM((DH + 8, TQ), F32),
            pltpu.VMEM((OFF, TQ), F32),
            pltpu.VMEM((DH, 8, TQ), F32),
            pltpu.VMEM((TM // NSPLIT, D), BF16),
            pltpu.VMEM((S, D), BF16),
            pltpu.VMEM((3, H, 128), F32),
            pltpu.VMEM((8, D), F32),
            pltpu.SMEM((1,), jnp.int32),
            pltpu.SemaphoreType.DMA((7,)),
            pltpu.SemaphoreType.DMA((NM,)),
            pltpu.SemaphoreType.DMA((S // TO,)),
        ],
        compiler_params=pltpu.CompilerParams(vmem_limit_bytes=100 * 1024 * 1024),
        name="preln_mha_swiglu",
    )(x, A_wqkv, A_wo, B_w1.T, B_w3.T, B_w2)
    return out.reshape(1, S, D)
```

```python
import jax
import jax.numpy as jnp
from jax import lax
import jax.experimental.pallas as pl
import jax.experimental.pallas.tpu as pltpu

S = 2048
D = 512
H = 32
DH = 16
F = 1376
EPS = 1e-5
LOG2E = 1.4426950408889634
QSCALE = (DH ** -0.5) * LOG2E

TQ = 512
NQ = S // TQ
KC = 128
NC = S // KC
LAG = 2
TM = 512
NM = S // TM
NSPLIT = 4
TO = 128
NG = D // 128
HG = 128 // DH

OFF = 16
KM = KC - OFF

SAFE_BOUND = 80.0
QN_HI = 2.0 ** 40
KN_HI = 2.0 ** 60
V_HI = 2.0 ** 30
V_LO = 2.0 ** -20
K_TINY = 2.0 ** -50

F32 = jnp.float32
BF16 = jnp.bfloat16
NT = (((1,), (1,)), ((), ()))


def _ln(x):
    m = jnp.mean(x, axis=-1, keepdims=True)
    xc = x - m
    v = jnp.mean(xc * xc, axis=-1, keepdims=True)
    return xc * lax.rsqrt(v + EPS)


def _dot(a, b):
    return jnp.dot(a, b, preferred_element_type=F32)


def _dot_nt(a, b):
    return lax.dot_general(a, b, NT, preferred_element_type=F32)


def _kernel(x_hbm, wqkv_hbm, wo_hbm, w1t_hbm, w3t_hbm, w2_hbm, out_hbm,
            x_v, wqkv_v, wo_v, w1t_v, w3t_v, w2_v,
            xn_s, k_s, rt_s, qt_s, vt_s, ot_s, cs_s, cp_s, cacc_s, va_s, qrow0_s, o0_s,
            out_v, stat_s, kmax_s, flag_s,
            w_sems, x_sems, out_sems):
    def x_copy(b):
        return pltpu.make_async_copy(x_hbm.at[pl.ds(b * TM, TM), :],
                                     x_v.at[pl.ds(b * TM, TM), :], x_sems.at[b])

    def w_copy(j):
        return pltpu.make_async_copy(wqkv_hbm.at[:, pl.ds(j * D, D)],
                                     wqkv_v.at[:, pl.ds(j * D, D)], w_sems.at[j])

    cp_x = [x_copy(b) for b in range(NM)]
    cp_w = [w_copy(j) for j in range(3)]
    cp_rest = [pltpu.make_async_copy(src, dst, w_sems.at[3 + i])
               for i, (src, dst) in enumerate(((wo_hbm, wo_v), (w1t_hbm, w1t_v),
                                               (w3t_hbm, w3t_v), (w2_hbm, w2_v)))]

    et_rows = lax.broadcasted_iota(jnp.int32, (H, D), 0)
    et_cols = lax.broadcasted_iota(jnp.int32, (H, D), 1) // DH
    et = jnp.where(et_rows == et_cols, 1.0, 0.0).astype(BF16)

    def rows(b):
        return pl.ds(pl.multiple_of(b * TM, TM), TM)

    def ln1(b):
        xn_s[rows(b), :] = _ln(x_v[rows(b), :].astype(F32)).astype(BF16)

    def run_max(slot, nrow, val):
        m = stat_s[slot, 0:nrow, :]
        for j in range(TM // 128):
            m = jnp.maximum(m, val[:, j * 128:(j + 1) * 128])
        stat_s[slot, 0:nrow, :] = m

    def proj_k(b):
        k = _dot(xn_s[rows(b), :], wqkv_v[:, D:2 * D])
        kb = k.astype(BF16)
        half = pl.ds(pl.multiple_of(b * (TM // 2), TM // 2), TM // 2)
        lane = lax.broadcasted_iota(jnp.int32, (OFF, 128), 1)
        for g in range(NG):
            kg = kb[:, g * 128:(g + 1) * 128]
            k_s[g, half, :] = pltpu.bitcast(kg, jnp.uint32)
            for j in range(TM // KC):
                kk = kg[j * KC + KM:(j + 1) * KC, :].astype(F32)
                kk = jnp.where(jnp.abs(kk) < K_TINY, K_TINY, kk)
                ratio = kk / pltpu.roll(kk, 1, 1)
                r0 = pl.multiple_of((b * (TM // KC) + j) * OFF, OFF)
                rt_s[g, pl.ds(r0, OFF), :] = jnp.where(lane % DH == 0, kk, ratio)
        kmax_s[...] = jnp.maximum(kmax_s[...], jnp.abs(k).reshape(TM // 8, 8, D).max(axis=0))

    def proj_q(b):
        qt = (_dot(xn_s[rows(b), :], wqkv_v[:, 0:D]) * QSCALE).T
        qt_s[b] = qt.astype(BF16)
        return (qt * qt).astype(BF16)

    def proj_v(b):
        vt = _dot(xn_s[rows(b), :], wqkv_v[:, 2 * D:3 * D]).T
        vt_s[b] = vt.astype(BF16)
        run_max(1, 8, jnp.abs(vt).reshape(D // 8, 8, TM).max(axis=0))

    def norm_q(qsq):
        run_max(0, H, _dot(et, qsq))

    cp_x[0].start()
    cp_w[1].start()
    stat_s[...] = jnp.zeros(stat_s.shape, F32)
    kmax_s[...] = jnp.zeros(kmax_s.shape, F32)
    cp_x[0].wait()
    cp_w[0].start()
    ln1(0)
    cp_w[1].wait()
    cp_w[2].start()
    cp_x[1].start()
    proj_k(0)
    cp_w[0].wait()
    cp_x[2].start()
    cp_x[3].start()
    qsq0 = proj_q(0)
    cp_w[2].wait()
    cp_x[1].wait()
    proj_v(0)
    norm_q(qsq0)
    ln1(1)
    cp_x[2].wait()
    cp_x[3].wait()
    for c in cp_rest:
        c.start()

    for b in range(1, NM):
        proj_k(b)
        qsq = proj_q(b)
        proj_v(b)
        norm_q(qsq)
        if b + 1 < NM:
            ln1(b + 1)

    zeros16 = jnp.zeros((DH, TQ), BF16)

    def head_weights(qb, g, hh):
        qh = qt_s[qb, pl.ds(pl.multiple_of(g * 128 + hh * DH, DH), DH), :]
        return qh, jnp.concatenate([zeros16] * hh + [qh] + [zeros16] * (HG - 1 - hh), axis=0)

    def probs(s, l):
        p = jnp.exp2(s)
        parts = [p[i * 8:(i + 1) * 8] for i in range(KC // 8)]
        m, v = parts[:KM // 8], parts[KM // 8:]
        for x in [v[0], m[0], v[1]] + m[1:]:
            l = l + x
        return p.astype(BF16), l

    def pv_dot(pb, row, c, acc):
        k0 = (c * KC) % TM
        vt = vt_s[(c * KC) // TM, pl.ds(row, DH), k0:k0 + KC]
        return acc + _dot(vt, pb)

    def pv_step(s, row, c, acc, l):
        pb, l = probs(s, l)
        return pv_dot(pb, row, c, acc), l

    def finish(slot, hh, acc, l):
        lsum = l.sum(axis=0, keepdims=True)
        ot_s[slot, hh * DH:(hh + 1) * DH, :] = acc * (1.0 / lsum)

    def tail(it_prev, slot_prev, last):
        row = pl.multiple_of((it_prev % NG) * 128 + (HG - 1) * DH, DH)
        acc = cacc_s[0:DH, :]
        l = cacc_s[DH:DH + 8, :]
        acc = pv_dot(pltpu.bitcast(cp_s[...], BF16), row, NC - 2, acc)
        last['acc'], last['l'] = acc, l
        yield None
        acc, l = pv_step(cs_s[...], row, NC - 1, acc, l)
        last['acc'], last['l'] = acc, l
        yield None
        finish(slot_prev, HG - 1, acc, l)
        yield None

    def q_rows(qh):
        qf = qh.astype(F32)
        return [jnp.broadcast_to(qf[d:d + 1, :], (8, TQ)) for d in range(DH)]

    def vpu_scores(g, c, hh, qr):
        r = rt_s[g, c * OFF:(c + 1) * OFF, :]
        a = [qr[DH - 1]] * (OFF // 8)
        for d in range(DH - 1, -1, -1):
            rb = jnp.broadcast_to(r[:, hh * DH + d:hh * DH + d + 1], (OFF, TQ))
            a = [a[u] * rb[u * 8:(u + 1) * 8] for u in range(OFF // 8)]
            if d > 0:
                a = [x + qr[d - 1] for x in a]
        return a

    def precompute(it):
        row = pl.multiple_of((it % NG) * 128, 128)
        qr = q_rows(qt_s[it // NG, pl.ds(row, DH), :])
        a = vpu_scores(it % NG, 0, 0, qr)
        for u in range(OFF // 8):
            va_s[u * 8:(u + 1) * 8, :] = a[u]
        for d in range(DH):
            qrow0_s[d] = qr[d]

    def b_body(it, carry):
        qb = it // NG
        g = it % NG
        items = [(hh, c) for hh in range(HG) for c in range(NC)]
        n = len(items)
        w = {}
        qrow = {}
        acc = {}
        l = {}
        s = {}
        last = {}

        def qk(i):
            hh, c = items[i]
            if hh not in w:
                qh, w[hh] = head_weights(qb, g, hh)
                qrow[hh] = [qrow0_s[d] for d in range(DH)] if hh == 0 else q_rows(qh)
            p0 = c * (KC // 2)
            km = pltpu.bitcast(k_s[g, p0:p0 + KM // 2, :], BF16)
            sm = _dot(km, w[hh])
            if i == 0:
                a = [va_s[u * 8:(u + 1) * 8, :] for u in range(OFF // 8)]
            else:
                a = vpu_scores(g, c, hh, qrow[hh])
            sc = jnp.concatenate([sm] + a, axis=0)
            if i == n - 1:
                cs_s[...] = sc
            else:
                s[i] = sc

        def pv(i):
            hh, c = items[i]
            row = pl.multiple_of(g * 128 + hh * DH, DH)
            if c == 0:
                l[hh] = (l[hh - 1] if hh > 0 else last['l']) * 0.0
                acc[hh] = (acc[hh - 1] if hh > 0 else last['acc']) * 0.0
            acc[hh], l[hh] = pv_step(s.pop(i), row, c, acc[hh], l[hh])
            if c == NC - 1:
                finish(it, hh, acc[hh], l[hh])

        prev = tail(jnp.maximum(it - 1, 0), jnp.where(it == 0, NQ * NG, it - 1), last)
        for j in range(n):
            qk(j)
            if j >= LAG:
                pv(j - LAG)
            else:
                next(prev)
                if j == LAG - 1:
                    next(prev)
        pb, l_last = probs(s.pop(n - 2), l[HG - 1])
        cp_s[...] = pltpu.bitcast(pb, jnp.uint32)
        cacc_s[0:DH, :] = acc[HG - 1]
        cacc_s[DH:DH + 8, :] = l_last
        precompute(jnp.minimum(it + 1, NQ * NG - 1))
        return carry

    precompute(0)
    cs_s[...] = jnp.zeros(cs_s.shape, F32)
    cp_s[...] = jnp.zeros(cp_s.shape, jnp.uint32)
    cacc_s[...] = jnp.zeros(cacc_s.shape, F32)
    lax.fori_loop(0, NQ * NG, b_body, 0)
    for _ in tail(NQ * NG - 1, NQ * NG - 1, {}):
        pass

    tr = TM // NSPLIT

    def o_piece(b, j):
        return ot_s[pl.ds(b * NG, NG), :, j * tr:(j + 1) * tr].reshape(D, tr).T.astype(BF16)

    o0_s[...] = o_piece(0, 0)

    kcol = jnp.max(kmax_s[...], axis=0, keepdims=True)
    kn = jnp.sum(jnp.where(et_rows == et_cols, kcol * kcol, 0.0), axis=1, keepdims=True)
    bound2 = kn * jnp.max(stat_s[0], axis=1, keepdims=True)
    bound2 = jnp.max(bound2) * 1.05
    vm = jnp.max(stat_s[1, 0:8, :])
    safe = jnp.logical_and(bound2 <= SAFE_BOUND * SAFE_BOUND,
                           jnp.logical_and(vm <= V_HI, vm >= V_LO))
    safe = jnp.logical_and(safe, jnp.logical_and(jnp.max(stat_s[0]) <= QN_HI,
                                                 jnp.max(kn) <= KN_HI))
    flag_s[0] = safe.astype(jnp.int32)

    @pl.when(flag_s[0] != 1)
    def _true_max_attention():
        head_rows = lax.broadcasted_iota(jnp.int32, (128, TQ), 0) // DH

        def body(it, carry):
            qb = it // H
            h = it % H
            g = h // HG
            hh = h % HG
            qg = qt_s[qb, pl.ds(pl.multiple_of(g * 128, 128), 128), :]
            w = jnp.where(head_rows == hh, qg, jnp.zeros_like(qg))
            row = pl.multiple_of(h * DH, DH)

            def scores(c):
                p0 = pl.multiple_of(c * (TM // 2), TM // 2)
                return _dot(pltpu.bitcast(k_s[g, pl.ds(p0, TM // 2), :], BF16), w)

            def max_pass(c, m):
                return jnp.maximum(m, jnp.max(scores(c), axis=0, keepdims=True))

            m = lax.fori_loop(0, NM, max_pass, jnp.full((1, TQ), -jnp.inf, F32))

            def sum_pass(c, al):
                acc, lsum = al
                p = jnp.exp2(scores(c) - m)
                return (acc + _dot(vt_s[c, pl.ds(row, DH), :], p.astype(BF16)),
                        lsum + jnp.sum(p, axis=0, keepdims=True))

            acc, lsum = lax.fori_loop(
                0, NM, sum_pass, (jnp.zeros((DH, TQ), F32), jnp.zeros((1, TQ), F32)))
            ot_s[qb * NG + g, pl.ds(pl.multiple_of(hh * DH, DH), DH), :] = acc * (1.0 / lsum)
            return carry

        lax.fori_loop(0, NQ * H, body, 0)
        o0_s[...] = o_piece(0, 0)

    for c in cp_rest:
        c.wait()

    def out_copy(b, j):
        r = pl.ds(pl.multiple_of(b * TM + j * TO, TO), TO)
        return pltpu.make_async_copy(out_v.at[r, :], out_hbm.at[r, :],
                                     out_sems.at[b * (TM // TO) + j])

    def c_body(b, carry):
        hs = []
        hns = []
        for j in range(NSPLIT):
            o = o0_s[...] if j == 0 else o_piece(b, j)
            xr = x_v[pl.ds(pl.multiple_of(b * TM + j * tr, tr), tr), :].astype(F32)
            hj = xr + _dot(o, wo_v[...])
            hs.append(hj)
            hns.append(_ln(hj).astype(BF16))
        h = jnp.concatenate(hs, axis=0)
        hn = jnp.concatenate(hns, axis=0)
        gate = _dot_nt(hn, w1t_v[...])
        up = _dot_nt(hn, w3t_v[...])
        a = (gate * jax.nn.sigmoid(gate) * up).astype(BF16)
        for j in range(TM // TO):
            y = h[j * TO:(j + 1) * TO] + _dot(a[j * TO:(j + 1) * TO], w2_v[...])
            out_v[pl.ds(pl.multiple_of(b * TM + j * TO, TO), TO), :] = y.astype(BF16)
            out_copy(b, j).start()
        o0_s[...] = o_piece(jnp.minimum(b + 1, NM - 1), 0)
        return carry

    lax.fori_loop(0, NM, c_body, 0)
    for b in range(NM):
        for j in range(TM // TO):
            out_copy(b, j).wait()


@jax.jit
def pallas_sequential_preLN__softmax_full_mha__glu_gated_swiglu__prompt_kernel(
    A_x: jax.Array,
    A_wqkv: jax.Array,
    A_wo: jax.Array,
    B_x: jax.Array,
    B_w1: jax.Array,
    B_w3: jax.Array,
    B_w2: jax.Array,
):
    del B_x
    x = A_x.reshape(S, D)
    hbm_spec = pl.BlockSpec(memory_space=pltpu.HBM)
    out = pl.pallas_call(
        _kernel,
        out_shape=jax.ShapeDtypeStruct((S, D), BF16),
        in_specs=[hbm_spec] * 6,
        out_specs=hbm_spec,
        scratch_shapes=[
            pltpu.VMEM((S, D), BF16),
            pltpu.VMEM((D, 3 * D), BF16),
            pltpu.VMEM((D, D), BF16),
            pltpu.VMEM((F, D), BF16),
            pltpu.VMEM((F, D), BF16),
            pltpu.VMEM((F, D), BF16),
            pltpu.VMEM((S, D), BF16),
            pltpu.VMEM((NG, S // 2, 128), jnp.uint32),
            pltpu.VMEM((NG, NC * OFF, 128), F32),
            pltpu.VMEM((NQ, D, TQ), BF16),
            pltpu.VMEM((NM, D, TM), BF16),
            pltpu.VMEM((NQ * NG + 1, 128, TQ), F32),
            pltpu.VMEM((KC, TQ), F32),
            pltpu.VMEM((KC // 2, TQ), jnp.uint32),
            pltpu.VMEM((DH + 8, TQ), F32),
            pltpu.VMEM((OFF, TQ), F32),
            pltpu.VMEM((DH, 8, TQ), F32),
            pltpu.VMEM((TM // NSPLIT, D), BF16),
            pltpu.VMEM((S, D), BF16),
            pltpu.VMEM((2, H, 128), F32),
            pltpu.VMEM((8, D), F32),
            pltpu.SMEM((1,), jnp.int32),
            pltpu.SemaphoreType.DMA((7,)),
            pltpu.SemaphoreType.DMA((NM,)),
            pltpu.SemaphoreType.DMA((S // TO,)),
        ],
        compiler_params=pltpu.CompilerParams(vmem_limit_bytes=100 * 1024 * 1024),
        name="preln_mha_swiglu",
    )(x, A_wqkv, A_wo, B_w1.T, B_w3.T, B_w2)
    return out.reshape(1, S, D)
```
